```python
import os as _os
_os.environ.setdefault("JAX_PLATFORMS", "cpu")
import jax
import jax.numpy as jnp

def _softmax(x, axis=-1):
    return jax.nn.softmax(x, axis=axis)
def _gelu(x):
    return jax.nn.gelu(x, approximate=True)
def _silu(x):
    return jax.nn.silu(x)
def _sigmoid(x):
    return jax.nn.sigmoid(x)
def _layernorm(x, axis=-1, eps=1e-5):
    m = jnp.mean(x, axis=axis, keepdims=True)
    v = jnp.var(x, axis=axis, keepdims=True)
    return (x - m) / jnp.sqrt(v + eps)
def _scatter_add(tgt, idx, src, axis=0):
    return tgt.at[idx].add(src)
def _segment_sum(src, seg, n):
    return jax.ops.segment_sum(src, seg, n)
class _Rng:
    def __init__(self, key):
        self._k = key
    def _next(self):
        self._k, sub = jax.random.split(self._k)
        return sub
    def normal(self, shape):
        return jax.random.normal(self._next(), shape, dtype=jnp.bfloat16)
    def randint(self, lo, hi, shape):
        return jax.random.randint(self._next(), shape, lo, hi, dtype=jnp.int32)
    def uniform(self, shape, lo=0.0, hi=1.0):
        return jax.random.uniform(self._next(), shape, jnp.bfloat16, lo, hi)
    def permutation(self, n):
        return jax.random.permutation(self._next(), n)


kernel_name = 'sequential_preLN__sliding_block__dense_activation_relu__prompt'

def setup_inputs():
    _rng = _Rng(jax.random.key(int.from_bytes(__import__("os").urandom(4), "little")))
    _w = (lambda a: (lambda t: t.astype(jnp.bfloat16) if jnp.issubdtype(t.dtype, jnp.floating) else t)(jnp.asarray(a)))
    def _A_setup():
        B, S, D = 1, 2048, 640
        return {
            "x": _w((lambda *s: _rng.normal(s) * 0.05)(B, S, D)),
            "wqkv": _w((lambda *s: _rng.normal(s) * 0.05)(D, 3 * D)),
            "wo": _w((lambda *s: _rng.normal(s) * 0.05)(D, D)),
        }
    _A_in = _A_setup()

    def _B_setup():
        B, S, D, Dff = 1, 2048, 640, 1536
        return {
            "x": _w((lambda *s: _rng.normal(s) * 0.05)(B, S, D)),
            "w1": _w((lambda *s: _rng.normal(s) * 0.05)(D, Dff)),
            "w2": _w((lambda *s: _rng.normal(s) * 0.05)(Dff, D)),
        }
    _B_in = _B_setup()

    return {
        "A_x": _A_in["x"],
        "A_wqkv": _A_in["wqkv"],
        "A_wo": _A_in["wo"],
        "B_x": _B_in["x"],
        "B_w1": _B_in["w1"],
        "B_w2": _B_in["w2"],
    }

def reference(A_x, A_wqkv, A_wo, B_x, B_w1, B_w2):
    def _A_ref(x, wqkv, wo):
        B, S, D = x.shape
        H = 32; Dh = D // H; W = 256
        qkv = (lambda x, *d: x.transpose(*d))((x @ wqkv).reshape(B, S, 3, H, Dh), 2, 0, 3, 1, 4)
        q, k, v = qkv[0], qkv[1], qkv[2]
        scores = jnp.einsum("bhqd,bhkd->bhqk", q, k) * (Dh ** -0.5)
        idx = jnp.arange(S)
        mask = (idx[:, None] - idx[None, :] >= 0) & (idx[:, None] - idx[None, :] < W)
        scores = jnp.where(mask[None, None], scores, -1e9)
        p = _softmax(scores, axis=-1)
        o = jnp.einsum("bhqk,bhkd->bhqd", p, v)
        return (lambda x, *d: x.transpose(*d))(o, 0, 2, 1, 3).reshape(B, S, D) @ wo

    def _B_ref(x, w1, w2):
        h = jnp.einsum("bsd,df->bsf", x, w1)
        zero = jnp.zeros_like(h)
        h = jnp.maximum(h, zero)
        return jnp.einsum("bsf,fd->bsd", h, w2)

    x = A_x
    h = x + _A_ref(_layernorm(x, axis=-1), A_wqkv, A_wo)
    h2 = h + _B_ref(_layernorm(h, axis=-1), B_w1, B_w2)
    return h2
```

```python
import contextlib
import functools
import numpy as np
import jax
import jax.numpy as jnp
from jax import lax
import jax.experimental.pallas as pl
import jax.experimental.pallas.tpu as pltpu

S, D, H, DH, DFF = 2048, 640, 32, 20, 1536
QB = 128
T = 2 * QB
NSTEP = S // T
RING = 4
EPS = 1e-5
LOG2E = 1.4426950408889634
BF16, F32, U32, I32 = jnp.bfloat16, jnp.float32, jnp.uint32, jnp.int32
ND, NF = D // 128, DFF // 128
partial = functools.partial


def _dot(a, b):
    return lax.dot_general(a, b, (((1,), (0,)), ((), ())), preferred_element_type=F32)


def _ln(x):
    m = jnp.mean(x, axis=-1, keepdims=True)
    c = x - m
    v = jnp.mean(c * c, axis=-1, keepdims=True)
    return c * lax.rsqrt(v + EPS)


def _upk(x):
    return pltpu.bitcast(x, BF16)


def _split(x):
    return [x[g:g + 8] for g in range(0, x.shape[0], 8)]


def _cat(xs):
    return xs[0] if len(xs) == 1 else jnp.concatenate(xs, axis=0)


def _structure(nk, nn):
    if nk == 5 and nn == 5:
        meth = [0, 0, 1, 1, 2]
        diag = [(i, i, meth[i]) for i in range(5)]
        return diag, [(i, j) for i in range(5) for j in range(i + 1, 5) if meth[i] != meth[j]]
    if nk == 5:
        diag = [(j % 5, j, j // 5) for j in range(10)]
        pairs = [(a, b) for a in range(5) for b in range(5, 10) if a != b % 5]
        if nn == 12:
            diag += [(0, 10, 0), (1, 11, 1), (2, 10, 0), (3, 11, 1)]
            pairs += [(10, 11), (12, 13)]
        return diag, pairs
    diag, pairs = _structure(nn, nk)
    pairs = sorted(pairs[:20], key=lambda ab: sorted((ab[0], ab[1] % 5))) + pairs[20:]
    return [(j, i, m) for i, j, m in diag], pairs


def _scheme(nk, nn, fast, rform=False):
    diag, pairs = _structure(nk, nn) if fast else ([], [])
    det = lambda s, t: 1 if (t - s) % 3 == 1 else -1
    dw, covered = {}, set()
    for e, (i, j, m) in enumerate(diag):
        a, b = (m + 1) % 3, (m + 2) % 3
        dw[e, a, b] = [(det(a, b), i, j)]
        dw[e, b, a] = [(-det(a, b), i, j)]
        covered.add((i, j))
    pp = []
    for e, e2 in pairs:
        (i, j, m), (i2, j2, m2) = diag[e], diag[e2]
        s, t, w = m2, m, 3 - m - m2
        sg = det(s, t)
        pp.append([([(1, s, i), (1, s, i2)], [(1, i2, j)], [(sg, t, j), (sg, t, j2)]),
                   ([(1, t, i), (1, t, i2)], [(1, i, j2)], [(-sg, s, j), (-sg, s, j2)]),
                   ([(1, s, i), (-1, t, i2)], [(1, i2, j), (-1, i, j2)], [(sg, s, j), (-sg, t, j2)])])
        dw[e, s, w].append((sg, i2, j))
        dw[e, w, s].append((-sg, i, j2))
        dw[e2, w, t].append((sg, i2, j))
        dw[e2, t, w].append((-sg, i, j2))
        covered |= {(i2, j), (i, j2)}
    dd = {e: [([(1, a, diag[e][0])], terms, [(1, b, diag[e][1])]) for (e1, a, b), terms in dw.items() if e1 == e]
          for e in range(len(diag))}
    slots = [[] for _ in pp]
    last = {e: max(n for n, pr in enumerate(pairs) if e in pr) for e in dd}
    for e in sorted(dd, key=lambda e: last[e]):
        col = diag[e][1]
        for p in dd[e]:
            touch = [n for n, pr in enumerate(pairs)
                     if not slots[n] and (e in pr or (nk > nn and col in (diag[pr[0]][1], diag[pr[1]][1])))]
            free = [n for n in range(last[e], -1, -1) if not slots[n]]
            slots[touch[-1] if touch else (free[0] if free else last[e])].append(p)
    prods = [p for n in range(len(pp)) for p in pp[n] + slots[n]]
    for j in range(nn):
        for i in range(nk):
            if (i, j) not in covered:
                prods.append(([(1, 0, i)], [(1, i, j)], [(1, 1, j)]))
                prods.append(([(1, 1, i)], [(1, i, j)], [(-1, 0, j)]))
    out = []
    for al, be, ga in prods:
        lhs = (((1, 0),), ((1, 1),), ((-1, 2),) if rform else ((-1, 0), (-1, 1)))
        rhs = (((-1, 1),), ((1, 0),), ((-1, 2),) if rform else ((-1, 0), (1, 1)))
        al = [(c * u, hf, i) for c, p, i in al for u, hf in lhs[p]]
        ga = [(c * u, hf, j) for c, p, j in ga for u, hf in rhs[p]]
        sa = al[0][0]
        al = [(c * sa, hf, i) for c, hf, i in al]
        sb = be[0][0] if len(be) == 1 else sa * ga[0][0]
        be = sorted([(c * sb, i, j) for c, i, j in be], reverse=True)
        ga = [(c * sa * sb, hf, j) for c, hf, j in ga]
        out.append((al, tuple(be), ga))
    return out


def _signed_sum(terms):
    first = next((n for n, (c, _) in enumerate(terms) if c > 0), None)
    sign = -1 if first is None else 1
    acc = terms[first or 0][1]
    for n, (c, v) in enumerate(terms):
        if n != (first or 0):
            acc = acc + v if c * sign > 0 else acc - v
    return sign, acc


BEATS = dict(d=16, q=36, p=9, x=0)


def make(LAG=1, TAIL=6, TAIL0=4, SCOPES=False, UNROLL=1, ONLY=None, NP=16, NACC=32, CH=2, SKIP=3, FRAC=0.8,
         AHEAD=1, ODELAY=80, RFORM=False, LN1W=(0.1, 0.9), LN2W=(60, 12), WQ=1, WP=1, FLAGS=None, EPI=1):
    scope = jax.named_scope if SCOPES else (lambda n: contextlib.nullcontext())
    jobs = dict(kq=(ND, 2 * ND), v=(ND, ND), o=(ND, ND), f1=(ND, NF), f2=(NF, ND))
    rform = dict(kq=False, v=RFORM, o=RFORM, f1=False, f2=False)
    schemes = {n: _scheme(*a, True, rform[n]) for n, a in jobs.items()}
    tile_of = {}
    for n, prods in schemes.items():
        for _, be, _ in prods:
            if len(be) > 1:
                tile_of.setdefault((n, be), len(tile_of))

    def kernel(x_h, wqkv_h, wo_h, w1_h, w2_h, out_h,
               x_v, out_v, wqkv, wo, w1, w2, wt, xn_s, k_s, krep, q_s, qt, v_s, vt, ot, o_s, h_s, hn_s, f_s, p_s,
               acc_s, sem_x, sem_w, sem_o, sem_b):
        def rows(i, off=0, n=T):
            r = i * T + off
            return pl.ds(r if isinstance(r, int) else pl.multiple_of(r, 16), n)

        def ocopy(i):
            return pltpu.make_async_copy(out_v.at[rows(i)], out_h.at[rows(i)], sem_o.at[i])

        def xcopy(j):
            r = pl.ds(j * T, T if j < 2 else S - 2 * T)
            return [pltpu.make_async_copy(x_h.at[r], x_v.at[r], sem_x.at[j])]

        def wcopy(j):
            src, dst, t0, t1 = ((wqkv_h, wqkv, ND, 2 * ND), (wqkv_h, wqkv, 0, ND), (wqkv_h, wqkv, 2 * ND, 3 * ND),
                                (wo_h, wo, 0, ND), (w1_h, w1, 0, NF), (w2_h, w2, 0, ND))[j]
            return [pltpu.make_async_copy(src.at[:, pl.ds(128 * t, 128)], dst.at[t], sem_w.at[j])
                    for t in range(t0, t1)]

        def start(copies):
            for c in copies:
                c.start()
            pl.semaphore_signal(sem_b)
            pl.semaphore_wait(sem_b)

        def wait(name, copies):
            with scope(name):
                for c in copies:
                    c.wait()

        sub8 = lax.broadcasted_iota(I32, (8, 128), 0)
        lane8 = lax.broadcasted_iota(I32, (8, 128), 1)

        def bits(cond):
            return jnp.where(cond, jnp.uint32(0xFFFFFFFF), jnp.uint32(0))

        def after(dep, val):
            never = jnp.abs(x_v[0:8, 0:128].astype(F32)) < -1.0
            return jnp.where(never, dep if dep.dtype == val.dtype else pltpu.bitcast(dep, val.dtype), val)

        def raw_tile(name, i, j, r0=0, n=128):
            if name == "kq":
                ref, j = wqkv, (j + ND) % (2 * ND)
            elif name == "v":
                ref, j = wqkv, j + 2 * ND
            else:
                ref = dict(o=wo, f1=w1, f2=w2)[name]
            return _upk(ref.bitcast(U32)[j, pl.ds((128 * i + r0) // 2, n // 2), :])

        def prep_tasks(name):
            def prep(be, idx, r0):
                _, w = _signed_sum([(c, raw_tile(name, i, j, r0, 16).astype(F32)) for c, i, j in be])
                wt[idx, r0:r0 + 16] = w.astype(BF16)
                return _split(w)
            return [(be, [partial(prep, be, idx, r0) for r0 in range(0, 128, 16)])
                    for (n, be), idx in tile_of.items() if n == name]

        nacc = [0]

        def matmul_ops(name, a_ref, done, init=None, raw=False):
            prods = _scheme(*jobs[name], False) if raw else schemes[name]
            left = {}
            for _, _, ga in prods:
                for j in {j for _, _, j in ga}:
                    left[j] = left.get(j, 0) + 1
            acc = {}

            def op(al, be, ga, pull, push):
                _, lhs = _signed_sum([(c, a_ref[hf, i]) for c, hf, i in al])
                w = raw_tile(name, *be[0][1:]) if len(be) == 1 else _upk(wt.bitcast(U32)[tile_of[name, be]])
                p = _dot(pull(lhs), w)
                push(p)
                for c, hf, j in ga:
                    if (hf, j) not in acc and init is not None and hf < 2:
                        acc[hf, j] = (1, init(hf, j))
                    if (hf, j) in acc:
                        c0, v = acc[hf, j]
                        acc[hf, j] = _signed_sum([(c0, acc_s[v] if isinstance(v, int) else v), (c, p)])
                    elif len(ga) == 1:
                        acc[hf, j] = (c, nacc[0] % NACC)
                        acc_s[nacc[0] % NACC] = p
                        nacc[0] += 1
                    else:
                        acc[hf, j] = (c, p)
                for j in sorted({j for _, _, j in ga}):
                    left[j] -= 1
                    if left[j] == 0:
                        get = lambda k, s: [(s * c, acc_s[v] if isinstance(v, int) else v)
                                            for c, v in ([acc[k]] if k in acc else [])]
                        for hf in range(2):
                            c, v = _signed_sum(get((hf, j), 1) + get((2, j), 1 - 2 * hf))
                            done(hf, j, v if c > 0 else -v)
            return [(name, p[1], partial(op, *p)) for p in prods]

        def ln_tasks(src, dst, step):
            def task(g):
                ys = [_ln(src(hf, g)) for hf in range(2)]
                if dst.shape[0] == 3:
                    ys.append(ys[0] + ys[1])
                for hf, y in enumerate(ys):
                    for t in range(ND):
                        dst[hf, t, g:g + step] = y[:, 128 * t:128 * t + 128]
                return [y[r:r + 8, 0:128] for y in ys[:2] for r in range(0, step, 8)]
            return [partial(task, g) for g in range(0, QB, step)]

        def ln1(i):
            return ln_tasks(lambda hf, g: x_v[rows(i, hf * QB + g, 8), :].astype(F32), xn_s.at[par(i)], 8)

        def slot(i, b):
            return (2 * i + b) % RING if isinstance(i, int) else (2 * i + b) & (RING - 1)

        def par(i):
            return int(isinstance(i, int) and i == 0)

        def kq_ops(i, raw=False):
            def done(hf, j, val):
                if j >= ND:
                    q_s[par(i), hf, j - ND] = (val * (DH ** -0.5 * LOG2E)).astype(BF16)
                else:
                    k_s[par(i), hf, j] = val.astype(BF16)
            return matmul_ops("kq", xn_s.at[par(i)], done, raw=raw)

        def v_ops(i, raw=False):
            def done(hf, j, val):
                v_s[par(i), hf, j] = val
            return matmul_ops("v", xn_s.at[par(i)], done, raw=raw)

        def relayout(i, b, h, dep):
            def gate(v):
                vs = _split(v)
                return v if dep is None else _cat([after(dep, vs[0])] + vs[1:])
            f0 = DH * h
            t0, t1 = f0 // 128, (f0 + DH - 1) // 128
            t = (16 * (f0 // 16) + 31) // 128
            if h == 0 or (16 * ((f0 - DH) // 16) + 31) // 128 < t:
                qt[b, pl.ds(64 * t, 64), :] = pltpu.bitcast(_upk(gate(q_s.bitcast(U32)[par(i), b, t])).T, U32)
                vt[slot(i, b), pl.ds(128 * t, 128), :] = gate(v_s[par(i), b, t]).T
            ku = k_s.bitcast(U32)
            lo = f0 % 128
            idx = (lo + ((lane8 - lo) & 31)) & 127
            for g in range(8):
                src = ku[par(i), b, t1, pl.ds(8 * g, 8), :]
                if t0 != t1:
                    src = jnp.where(lane8 >= 64, ku[par(i), b, t0, pl.ds(8 * g, 8), :], src)
                krep[slot(i, b), h, pl.ds(8 * g, 8), :] = jnp.take_along_axis(gate(src), idx, axis=1)

        def nblk(i, b):
            return min(2 * i + b + 1, 3) if isinstance(i, int) else 3

        def qk(i, b, h):
            n = nblk(i, b)
            f0 = DH * h
            v0 = f0 // 16
            lo = f0 - 16 * v0
            qa = qt[b, 8 * v0:8 * v0 + 8, :]
            qb = qt[b, 8 * v0 + 8:8 * v0 + 16, :]
            if lo > 0:
                qa = qa & bits(sub8 >= lo // 2)
            if lo + DH < 32:
                qb = qb & bits(sub8 < (lo + DH - 16) // 2)
            parts = [None] * 8
            for a in range(4):
                cm = bits((lane8 >> 5) == a)
                parts[(v0 + 2 * a) % 8] = qa & cm
                parts[(v0 + 2 * a + 1) % 8] = qb & cm
            kb = [krep[slot(i, b + 1 - n + j), h] for j in range(n)]
            if n == 3:
                d = (lane8 - f0 % 128) & 127
                ka, kc = _split(kb[0]), _split(kb[2])
                main = [jnp.where(d >= 32 * (g // 2 + 1), kc[g], ka[g]) for g in range(6)] + ka[6:]
                ext = []
                for g in range(2):
                    e = kc[g]
                    for a in range(1, 4):
                        e = jnp.where(d >= 32 * a, kc[2 * a + g], e)
                    ext.append(e)
                kb = ext + main + [kb[1]]
            return _dot(_upk(_cat(kb)), _upk(_cat(parts)))

        def softmax_tasks(i, b, h, s, buf):
            n = nblk(i, b)
            rel = lane8 - sub8
            s = _split(s)
            if n == 3:
                sm = [jnp.where(jnp.where((lane8 >> 5) == g // 4, rel, -1) >= 8 * g, s[g % 4], s[4 + g])
                      for g in range(16)] + s[20:]
            else:
                sm = [jnp.where(rel >= 8 * g, s[16 * (n - 1) + g], -1e30) for g in range(16)] + s[:16 * (n - 1)]
            m = jnp.max(functools.reduce(jnp.maximum, sm), axis=0, keepdims=True)
            m = [jnp.broadcast_to(m, (8, 128))]

            def task(g, dep):
                if dep is not None:
                    m[0] = after(dep, m[0])
                p_s[buf, 8 * g:8 * (g + CH)] = _cat([jnp.exp2(v - m[0]) for v in sm[g:g + CH]]).astype(BF16)
            return [partial(task, g) for g in range(0, len(sm), CH)]

        def pv(i, b, h, buf):
            n = nblk(i, b)
            f0 = DH * h
            pu = p_s.bitcast(U32)
            ps = [pu[buf, 64 * j:64 * j + 64] for j in range(min(n, 2))][::-1]
            if n == 3:
                r2 = lax.broadcasted_iota(I32, (QB // 2, QB), 0) * 2
                c2 = lax.broadcasted_iota(I32, (QB // 2, QB), 1)
                tri_bits = (jnp.where(r2 <= c2, jnp.uint32(0xFFFF), jnp.uint32(0))
                            | jnp.where(r2 + 1 <= c2, jnp.uint32(0xFFFF0000), jnp.uint32(0)))
                pc = ps[1] & tri_bits
                ps = [ps[1] ^ pc, ps[0], pc]
            o = None
            for j in range(n):
                r0 = f0 // 8 * 8
                vs = [vt[slot(i, b + 1 - n + j), r0 + 8 * g:r0 + 8 * g + 8, :] for g in range(3)]
                if f0 % 8 == 0:
                    vs[2] = jnp.where(sub8 >= 4, 1.0, vs[2])
                else:
                    vs[0] = jnp.where(sub8 < 4, 1.0, vs[0])
                r = _dot(_cat(vs), _upk(ps[j]))
                o = r if o is None else o + r
            l = jnp.broadcast_to(o[23:24] if f0 % 8 == 0 else o[0:1], (8, 128))
            inv = pl.reciprocal(l, approx=True)
            inv = inv * (2.0 - l * inv)
            return [v * inv for v in _split(o)]

        def o_ops(i, raw=False):
            def done(hf, j, val):
                h_s[hf, :, 128 * j:128 * j + 128] = val
            return matmul_ops("o", o_s.at[par(i)], done,
                              lambda hf, j: x_v[rows(i, hf * QB, QB), 128 * j:128 * j + 128].astype(F32), raw)

        def ln2():
            return ln_tasks(lambda hf, g: h_s[hf, g:g + 8, :], hn_s, 8)

        def ffn_ops(i):
            def done1(hf, j, val):
                f_s[hf, j] = jnp.maximum(val, 0.0)

            def done2(hf, j, val):
                out_v[rows(i, hf * QB, QB), 128 * j:128 * j + 128] = val.astype(out_v.dtype)
            return (matmul_ops("f1", hn_s, done1)
                    + matmul_ops("f2", f_s, done2, lambda hf, j: h_s[hf, :, 128 * j:128 * j + 128]))

        def units(ops):
            return [("d", ops[j:j + 4]) for j in range(0, len(ops), 4)]

        def with_attention(i, dense, tail):
            seq = []
            for g in range(H // 2 + LAG):
                if g < H // 2:
                    seq.append((WQ, ("q", (i, g))))
                if g >= LAG:
                    seq.append((WP, ("p", (i, g - LAG))))
            total = len(dense) - tail
            wsum = sum(w for w, _ in seq[:-1])
            done, acc, plan = 0, 0.0, []
            for w, e in seq:
                plan.append(e)
                acc += w
                while done < min(total * acc / wsum - 0.5, total):
                    plan.append(dense[done])
                    done += 1
            return plan + dense[done:]

        class Plan:
            def __init__(self, plan):
                self.plan = plan
                self.t0 = [0]
                for kind, _ in plan:
                    self.t0.append(self.t0[-1] + BEATS[kind])
                self.pulls = []

            def first(self, name, be=None):
                return next(t for (kind, u), t in zip(self.plan, self.t0)
                            if kind == "d" and any(o[0] == name and be in (None, o[1]) for o in u))

            def last(self, name):
                return max(t + 16 for (kind, u), t in zip(self.plan, self.t0)
                           if kind == "d" and any(o[0] == name for o in u))

            def spread(self, tasks, t0, t1):
                for n, fn in enumerate(tasks):
                    self.pulls.append((t0 + (t1 - t0) * n / len(tasks), fn))

            def prep(self, name, t0, t1):
                tasks = prep_tasks(name)
                t = t1
                for be, fns in tasks[::-1]:
                    if any(k == "d" and any(o[:2] == (name, be) for o in u) for k, u in self.plan):
                        t = min(t, self.first(name, be) - 12)
                    dt = (t1 - t0) * (len(be) + 1) / sum(len(b) + 1 for b, _ in tasks)
                    self.spread(fns, max(t - dt, t0), max(t, t0))
                    t -= dt

            def run(self):
                queue, rate, score, outs = [], [0.0, 0.0, 0], [None], {}
                dense_end = max(t + 15 for (kind, _), t in zip(self.plan, self.t0) if kind == "d")

                def push(val):
                    for dep in _split(val):
                        if rate[2] > 0:
                            rate[2] -= 1
                            continue
                        rate[1] += rate[0]
                        while queue and rate[1] >= 1:
                            rate[1] -= 1
                            queue.pop(0)[1](dep)

                for n, (kind, u) in enumerate(self.plan):
                    t0 = self.t0[n]
                    if kind == "x":
                        u()
                    elif kind == "d":
                        due = sorted((e for e in self.pulls if min(e[0], dense_end) < t0 + 16), key=lambda e: e[0])
                        self.pulls = [e for e in self.pulls if min(e[0], dense_end) >= t0 + 16]
                        deps = [(min(max(int(t - t0), 0), 15), dep) for t, fn in due for dep in fn()]

                        def pull(lhs):
                            vs = _split(lhs)
                            for g, dep in deps:
                                vs[g] = after(dep, vs[g])
                            return _cat(vs)
                        for j, (_, _, op) in enumerate(u):
                            op(pull if j == 0 else (lambda v: v), push if j == 0 else (lambda v: None))
                    elif kind == "q":
                        i, g = u
                        for gg in ([g + AHEAD] if g > 0 else range(AHEAD + 1)):
                            for h in range(2 * gg, min(2 * gg + 2, H)):
                                for b in range(2):
                                    relayout(i, b, h, score[0])
                        new = []
                        for j, (b, h) in enumerate((b, h) for b in range(2) for h in (2 * g, 2 * g + 1)):
                            s = qk(i, b, h)
                            if j == 3:
                                push(s)
                            score[0] = s[0:8]
                            new += softmax_tasks(i, b, h, s, (4 * g + j) % NP)
                        queue.extend((g, fn) for fn in new)
                        end = next(m for m, e in enumerate(self.plan) if e[0] == "p" and e[1][1] == g and m > n)
                        ticks = -SKIP
                        for k, _ in self.plan[n + 1:end - 1]:
                            ticks += dict(d=16, q=16 * nblk(i, 1), p=0, x=0)[k]
                            if k == "q":
                                break
                        rate[:] = [len(queue) / max(ticks * FRAC, 1), 0.0, SKIP]
                    else:
                        i, g = u
                        while queue and queue[0][0] <= g:
                            queue.pop(0)[1](None)
                        for b in range(2):
                            a, e = [pv(i, b, 2 * g + j, (4 * g + 2 * b + j) % NP) for j in range(2)]
                            ot[b, 40 * g:40 * g + 40, :] = _cat([a[0], a[1], jnp.where(sub8 < 4, a[2], e[0]), e[1], e[2]])
                        t = 40 * (g + 1) // 128 - 1
                        if t >= 0 and 40 * g < 128 * (t + 1):
                            vals = [ot[b, 128 * t:128 * t + 128, :].T for b in range(2)]
                            if o_s.shape[1] == 3:
                                vals.append(vals[0] + vals[1])
                            for b, val in enumerate(vals):
                                o_s[par(i), b, t] = val
                            self.pulls.append((t0 + ODELAY, partial(lambda vs: [v[QB - 8:] for v in vs], vals[:2])))
                assert not self.pulls

        def prologue():
            start(xcopy(0))
            start(wcopy(0))
            start(wcopy(1))
            start(wcopy(2) + xcopy(1))
            start(wcopy(3) + wcopy(4))
            start(wcopy(5))
            start(xcopy(2))
            wait("wx0", xcopy(0))
            for fn in ln1(0):
                fn()
            wait("wk", wcopy(0))
            kq0 = kq_ops(0, raw=True)
            a1 = with_attention(0, units(kq_ops(1) + v_ops(1)), TAIL0)
            c0 = with_attention(1, units(ffn_ops(0)), TAIL)
            plan = (units(kq0[:48]) + [("x", partial(wait, "wq", wcopy(1)))]
                    + units(kq0[48:]) + [("x", partial(wait, "wv", wcopy(2) + xcopy(1)))]
                    + units(v_ops(0, raw=True)) + a1[:W1AT] + [("x", partial(wait, "w1", wcopy(3) + wcopy(4)))]
                    + a1[W1AT:] + units(o_ops(0, raw=True)) + c0[:W2AT]
                    + [("x", partial(wait, "w2", wcopy(5) + xcopy(2)))] + c0[W2AT:])
            p = Plan(plan)
            bar = [t for (kind, _), t in zip(p.plan, p.t0) if kind == "x"]
            p.prep("kq", bar[0], bar[1] + 16 * 12)
            p.prep("v", bar[1] + 16 * 13, p.last("v"))
            p.prep("f1", bar[2], p.last("f1"))
            p.prep("f2", bar[3], p.last("f2"))
            p.prep("o", p.first("f2"), p.last("f2"))
            p.spread(ln1(1), bar[1] + 50, bar[1] + 16 * 13 - 1)
            p.spread(ln2(), p.first("f1"), p.first("f1"))
            p.spread(ln1(2), p.first("f1") + 60, p.last("f2") - 60)
            p.run()
            ocopy(0).start()

        W1AT, W2AT = 46, 12
        if ONLY in (None, "pro"):
            prologue()

        def steps(i0, n):
            plan, marks = [], []
            for i in [i0 + j for j in range(n)]:
                marks.append(len(plan))
                plan += units(o_ops(i - 1) + kq_ops(i) + v_ops(i))
                marks.append(len(plan))
                plan += with_attention(i, units(ffn_ops(i - 1)), TAIL)
            p = Plan(plan)
            marks = [p.t0[m] for m in marks] + [p.t0[-1]]
            for j in range(n):
                a, b, c = marks[2 * j:2 * j + 3]
                p.spread(ln2(), a + 16 * 11 + LN2W[0], a + 16 * 11 + LN2W[0] + 32 * LN2W[1])
                p.spread(ln1(jnp.minimum(i0 + j + 1, NSTEP - 1)), b + (c - b) * LN1W[0], b + (c - b) * LN1W[1])
            p.run()
            for j in range(n):
                ocopy(i0 + j - 1).start()

        def step(it, carry):
            steps(2 + it * UNROLL, UNROLL)
            return carry

        if ONLY in (None, "loop"):
            with scope("loop"):
                lax.fori_loop(0, (NSTEP - 2) // UNROLL, step, 0)
        if ONLY not in (None, "epi"):
            def keep(i, c):
                for r in (v_s, xn_s, ot, o_s, h_s, hn_s, f_s, vt, acc_s):
                    rr = r.at[i] if len(r.shape) == 3 else (r.at[i, 0] if len(r.shape) == 4 else r.at[i, 0, 0])
                    out_v[0:16, 0:128] += rr[0:16, 0:128].astype(BF16)
                    rr[0:16, 0:128] = out_v[0:16, 0:128].astype(F32)
                for r in (k_s, q_s, p_s, wt):
                    rr = r.at[i] if len(r.shape) == 3 else r.at[i, 0, 0]
                    out_v[0:16, 0:128] += rr[0:16, 0:128]
                    rr[0:16, 0:128] = out_v[0:16, 0:128]
                return c
            lax.fori_loop(0, 2, keep, 0)
            ocopy(1).start()
            ocopy(1).wait()
            return

        p = Plan(units(o_ops(NSTEP - 1)) + units(ffn_ops(NSTEP - 1)))
        p.spread(ln2(), p.first("f1"), p.first("f1") + 16)
        p.run()
        ocopy(NSTEP - 1).start()
        wait("wout", [ocopy(i) for i in range(NSTEP)])

    def fn(A_x, A_wqkv, A_wo, B_x, B_w1, B_w2):
        del B_x
        x = A_x.reshape(S, D)
        any_spec = pl.BlockSpec(memory_space=pl.ANY)
        nh = 3 if RFORM else 2
        out = pl.pallas_call(
            kernel,
            in_specs=[any_spec] * 5,
            out_specs=any_spec,
            out_shape=jax.ShapeDtypeStruct((S, D), A_x.dtype),
            scratch_shapes=[
                pltpu.VMEM((S, D), BF16), pltpu.VMEM((S, D), BF16),
                pltpu.VMEM((3 * ND, D, 128), BF16), pltpu.VMEM((ND, D, 128), BF16),
                pltpu.VMEM((NF, D, 128), BF16), pltpu.VMEM((ND, DFF, 128), BF16),
                pltpu.VMEM((len(tile_of), 128, 128), BF16),
                pltpu.VMEM((2, nh, ND, QB, 128), F32),
                pltpu.VMEM((2, 2, ND, QB, 128), BF16),
                pltpu.VMEM((RING, H, QB // 2, 128), U32),
                pltpu.VMEM((2, 2, ND, QB, 128), BF16),
                pltpu.VMEM((2, D // 2, 128), U32),
                pltpu.VMEM((2, 2, ND, QB, 128), F32),
                pltpu.VMEM((RING, D, 128), F32),
                pltpu.VMEM((2, D, 128), F32),
                pltpu.VMEM((2, nh, ND, QB, 128), F32),
                pltpu.VMEM((2, QB, D), F32),
                pltpu.VMEM((2, ND, QB, 128), F32),
                pltpu.VMEM((2, NF, QB, 128), F32),
                pltpu.VMEM((NP, 2 * QB, 128), BF16),
                pltpu.VMEM((NACC, QB, 128), F32),
                pltpu.SemaphoreType.DMA((3,)),
                pltpu.SemaphoreType.DMA((6,)),
                pltpu.SemaphoreType.DMA((NSTEP,)),
                pltpu.SemaphoreType.REGULAR,
            ],
            compiler_params=pltpu.CompilerParams(vmem_limit_bytes=100 * 1024 * 1024, flags=FLAGS),
            name="fused_block",
        )(x, A_wqkv, A_wo, B_w1, B_w2)
        return out.reshape(1, S, D)
    return fn


_impl = make()


@jax.jit
def pallas_sequential_preLN__sliding_block__dense_activation_relu__prompt_kernel(A_x, A_wqkv, A_wo, B_x, B_w1, B_w2):
    return _impl(A_x, A_wqkv, A_wo, B_x, B_w1, B_w2)
```

```python
import functools

import jax
import jax.experimental.pallas as pl
import jax.experimental.pallas.tpu as pltpu
import jax.numpy as jnp
import numpy as np
from jax import lax

S, D, H, DH, DFF = 2048, 640, 32, 20, 1536
QB = 128
T = 2 * QB
NSTEP = S // T
ND, NF = D // 128, DFF // 128
RING = 4
CUTS = (0, 24, 48, 72, 96, 112)
NBUF = 16
EPS = 1e-5
QSCALE = DH ** -0.5 * 1.4426950408889634
BF16, F32, U32, I32 = jnp.bfloat16, jnp.float32, jnp.uint32, jnp.int32
partial = functools.partial


def _scheme(nk, nn, diag=(), pairs=()):
    pts = np.array([[1, 0], [0, 1], [-1, -1]])
    perp = np.array([[0, -1], [1, 0], [-1, 1]])
    ek, en = np.eye(nk, dtype=int), np.eye(nn, dtype=int)
    els, prods, covered = [], [], np.zeros((nk, nn), bool)
    for i, j, m in diag:
        s, t = (m + 1) % 3, (m + 2) % 3
        els.append((ek[i], en[j], m))
        prods += [(np.outer(pts[s], ek[i]), np.outer(perp[t], en[j])),
                  (np.outer(pts[t], ek[i]), np.outer(perp[s], en[j]))]
        covered[i, j] = True
    for e, e2 in pairs:
        (a, c, t), (a2, c2, s) = els[e], els[e2]
        prods += [(np.outer(pts[s], a + a2), np.outer(perp[t], c + c2)),
                  (np.outer(pts[t], a + a2), np.outer(perp[s], c + c2)),
                  (np.outer(pts[s], a) - np.outer(pts[t], a2), np.outer(perp[s], c) - np.outer(perp[t], c2))]
        els.append((a + a2, c + c2, 3 - s - t))
        covered |= (np.outer(a, c2) + np.outer(a2, c)) != 0
    for j in range(nn):
        for i in range(nk):
            if not covered[i, j]:
                prods += [(np.outer(pts[hf], ek[i]), np.outer(pts[hf], en[j])) for hf in range(2)]
    lhs = np.stack([np.kron(a.ravel(), c.ravel()) for a, c in prods], axis=1)
    rhs = np.einsum("hg,ik,jl->higjkl", np.eye(2, dtype=int), ek, en).reshape(lhs.shape[0], -1)
    w = np.rint(np.linalg.lstsq(lhs.astype(float), rhs.astype(float), rcond=None)[0]).astype(int)
    assert np.array_equal(lhs @ w, rhs) and max(np.abs(lhs).max(), np.abs(w).max()) == 1

    def terms(m, sign):
        return tuple((int(sign * m[r, c]), int(r), int(c)) for r, c in zip(*np.nonzero(m)))

    out = []
    for (a, c), b in zip(prods, w.reshape(-1, nk, nn)):
        sa, sb = a[a != 0][0], b[b != 0][0]
        out.append((terms(a, sa), terms(b, sb), terms(c, sa * sb)))
    return out


ORDER = dict(
    kq=[43, 55, 41, 18, 38, 68, 32, 77, 39, 36, 27, 24, 44, 56, 65, 53, 40, 26, 16, 28, 33, 34, 42, 3, 54, 21, 48,
        30, 22, 25, 20, 23, 0, 29, 31, 1, 71, 73, 8, 59, 51, 50, 5, 52, 66, 19, 67, 7, 45, 46, 58, 57, 4, 47, 49,
        12, 78, 9, 79, 17, 37, 35, 14, 2, 72, 61, 60, 13, 11, 10, 70, 69, 62, 63, 64, 6, 74, 75, 15, 76],
    v=[25, 35, 9, 16, 20, 23, 14, 11, 17, 18, 34, 36, 3, 27, 26, 2, 32, 33, 31, 37, 12, 0, 4, 10, 22, 24, 19, 21,
       13, 6, 1, 15, 38, 8, 7, 39, 30, 5, 29, 28],
    o=[0, 36, 17, 34, 11, 12, 1, 4, 38, 31, 28, 8, 15, 14, 24, 23, 19, 22, 10, 13, 37, 29, 39, 30, 5, 20, 21, 3, 9,
       16, 35, 18, 33, 6, 7, 32, 26, 2, 25, 27],
    ffn=[82, 79, 28, 31, 84, 83, 33, 32, 46, 58, 40, 52, 80, 81, 56, 57, 66, 6, 64, 69, 70, 12, 67, 55, 74, 62, 53,
         65, 90, 93, 92, 89, 35, 5, 59, 54, 68, 30, 29, 13, 22, 97, 88, 91, 8, 76, 77, 78, 7, 71, 72, 15, 37, 75,
         18, 73, 26, 27, 23, 96, 85, 86, 87, 9, 1, 19, 38, 39, 4, 63, 61, 60, 44, 45, 43, 14, 41, 10, 11, 42, 36,
         0, 16, 34, 48, 3, 47, 17, 51, 50, 49, 2, 21, 194, 107, 94, 20, 95, 25, 24, 153, 167, 170, 110, 132, 126,
         162, 165, 121, 179, 111, 120, 112, 131, 187, 143, 118, 98, 128, 188, 119, 130, 151, 123, 129, 150, 186,
         138, 182, 195, 106, 180, 159, 147, 141, 177, 168, 124, 189, 156, 192, 174, 176, 108, 166, 142, 145, 169,
         178, 101, 149, 148, 144, 100, 146, 114, 136, 172, 184, 175, 139, 134, 127, 99, 191, 161, 158, 193, 137,
         135, 173, 116, 181, 157, 160, 190, 155, 152, 140, 154, 102, 113, 122, 103, 171, 117, 183, 185, 164, 133,
         163, 109, 115, 105, 125, 104])
SHAPES = dict(kq=(ND, 2 * ND), v=(ND, ND), o=(ND, ND), f1=(ND, NF), f2=(NF, ND))


def _schemes():
    d10 = [(j % 5, j, j // 5) for j in range(10)]
    p10 = [(a, b) for a in range(5) for b in range(5, 10) if a != b - 5]
    d12 = d10 + [(0, 10, 0), (1, 11, 1), (2, 10, 0), (3, 11, 1)]
    p12 = p10 + [(10, 11), (12, 13)]
    d5 = [(i, i, (0, 0, 1, 1, 2)[i]) for i in range(5)]
    p5 = [(0, 2), (0, 3), (0, 4), (1, 2), (1, 3), (1, 4), (2, 4), (3, 4), (7, 1), (11, 3)]
    kq, sq = _scheme(5, 10, d10, p10), _scheme(5, 5, d5, p5)
    f1, f2 = _scheme(5, 12, d12, p12), _scheme(12, 5, [(j, i, m) for i, j, m in d12], p12)
    assert all(sorted(ORDER[n]) == list(range(len(p)))
               for n, p in (("kq", kq), ("v", sq), ("o", sq), ("ffn", f1 + f2)))
    return dict(kq=[kq[j] for j in ORDER["kq"]], v=[sq[j] for j in ORDER["v"]], o=[sq[j] for j in ORDER["o"]],
                f1=[f1[j] for j in ORDER["ffn"] if j < len(f1)],
                f2=[f2[j - len(f1)] for j in ORDER["ffn"] if j >= len(f1)])


SCHEMES = _schemes()
WEIGHT_SUMS = {}
for _name, _prods in SCHEMES.items():
    for _, _beta, _ in _prods:
        if len(_beta) > 1:
            WEIGHT_SUMS.setdefault((_name, _beta), len(WEIGHT_SUMS))


def _dot(a, b):
    return lax.dot_general(a, b, (((1,), (0,)), ((), ())), preferred_element_type=F32)


def _layernorm(x):
    c = x - jnp.mean(x, axis=-1, keepdims=True)
    return c * lax.rsqrt(jnp.mean(c * c, axis=-1, keepdims=True) + EPS)


def _unpack(x):
    return pltpu.bitcast(x, BF16)


def _split(x):
    return [x[g:g + 8] for g in range(0, x.shape[0], 8)]


def _cat(xs):
    return xs[0] if len(xs) == 1 else jnp.concatenate(xs, axis=0)


def _signed_sum(terms):
    first = next((n for n, (c, _) in enumerate(terms) if c > 0), None)
    sign = -1 if first is None else 1
    acc = terms[first or 0][1]
    for n, (c, v) in enumerate(terms):
        if n != (first or 0):
            acc = acc + v if c * sign > 0 else acc - v
    return sign, acc


def _kernel(x_hbm, wqkv_hbm, wo_hbm, w1_hbm, w2_hbm, out_hbm,
            x_s, out_s, wqkv_s, wo_s, w1_s, w2_s, wsum_s, xn_s, xnext_s, k_s, q_s, v_s, krep_s, qt_s, qmask_s, vt_s,
            s_s, p_s, ot_s, o_s, h_s, hn_s, f_s, acc_s, sem_x, sem_w, sem_o, sem_order):
    sub8 = lax.broadcasted_iota(I32, (8, 128), 0)
    lane8 = lax.broadcasted_iota(I32, (8, 128), 1)

    def rows(i, off=0, n=T):
        r = i * T + off
        return pl.ds(r if isinstance(r, int) else pl.multiple_of(r, 16), n)

    def first(i):
        return int(isinstance(i, int) and i == 0)

    def after(dep, val):
        never = qmask_s[0] == 1
        return jnp.where(never, dep if dep.dtype == val.dtype else pltpu.bitcast(dep, val.dtype), val)

    def x_copies(j):
        r = pl.ds(j * T, T if j < 3 else S - 3 * T)
        return [pltpu.make_async_copy(x_hbm.at[r], x_s.at[r], sem_x.at[j])]

    def w_copies(j):
        src, dst, t0, t1 = ((wqkv_hbm, wqkv_s, 2 * ND, 2 * ND + 1), (wqkv_hbm, wqkv_s, 2 * ND + 1, 2 * ND + 3),
                            (wqkv_hbm, wqkv_s, 2 * ND + 3, 3 * ND), (wqkv_hbm, wqkv_s, ND, 2 * ND),
                            (wqkv_hbm, wqkv_s, 0, ND), (wo_hbm, wo_s, 0, ND), (w1_hbm, w1_s, 0, NF),
                            (w2_hbm, w2_s, 0, ND))[j]
        return [pltpu.make_async_copy(src.at[:, pl.ds(128 * t, 128)], dst.at[t], sem_w.at[j]) for t in range(t0, t1)]

    def out_copy(i):
        return pltpu.make_async_copy(out_s.at[rows(i)], out_hbm.at[rows(i)], sem_o.at[i])

    def last_out_copy(j):
        win = (rows(NSTEP - 1), pl.ds(128 * j, 128))
        return pltpu.make_async_copy(out_s.at[win], out_hbm.at[win], sem_o.at[NSTEP - 1])

    def wait(copies):
        for c in copies:
            c.wait()

    def weight(name, i, j, r0=0, n=128):
        if name == "kq":
            ref, j = wqkv_s, (j + ND) % (2 * ND)
        elif name == "v":
            ref, j = wqkv_s, j + 2 * ND
        else:
            ref = dict(o=wo_s, f1=w1_s, f2=w2_s)[name]
        return _unpack(ref.bitcast(U32)[j, pl.ds((128 * i + r0) // 2, n // 2), :])

    def weight_sum_tasks(name):
        groups = []
        for beta in sorted((b for n, b in WEIGHT_SUMS if n == name), key=lambda b: -len(b)):
            src = {t[1:] for t in beta}
            best = max(groups, key=lambda g: len(g[0] & src), default=None)
            if best is not None and best[0] & src and len(best[0] | src) <= 9:
                best[0].update(src)
                best[1].append(beta)
            else:
                groups.append((src, [beta]))

        def task(beta, r0):
            _, w = _signed_sum([(c, weight(name, i, j, r0, 16).astype(F32)) for c, i, j in beta])
            wsum_s[WEIGHT_SUMS[name, beta], r0:r0 + 16] = w.astype(BF16)
            return _split(w)

        return [(len(src) + sum(map(len, betas)), betas,
                 [partial(task, beta, r0) for r0 in range(0, 128, 16) for beta in betas]) for src, betas in groups]

    class Matmul:
        def __init__(self, name, a_ref, done, init=None, prods=None):
            self.name, self.a_ref, self.done, self.init = name, a_ref, done, init
            self.prods = prods or SCHEMES[name]
            self.unit = [0] * len(self.prods)
            self.last = {j: n for n, (_, _, gamma) in enumerate(self.prods) for _, _, j in gamma}
            self.acc = {}

        def ops(self):
            return [(self, n) for n in range(len(self.prods))]

        def slot(self, hf, j):
            return hf, j + (NF if self.name == "f2" else 0)

        def load(self, hf, j, rs):
            c, v = self.acc.get((hf, j, rs.start)) or self.acc[hf, j, 0]
            return c, (acc_s[self.slot(hf, j) + (rs,)] if v is None else v)

        def run(self, n, rs, pull):
            alpha, beta, gamma = self.prods[n]
            _, lhs = _signed_sum([(c, self.a_ref[hf, i, rs]) for c, hf, i in alpha])
            if len(beta) == 1:
                w = weight(self.name, *beta[0][1:])
            else:
                w = _unpack(wsum_s.bitcast(U32)[WEIGHT_SUMS[self.name, beta]])
            p = _dot(pull(lhs), w)
            for c, hf, j in gamma:
                uses = [m for m, (_, _, g) in enumerate(self.prods) if any((hf, j) == t[1:] for t in g)]
                if uses[0] < n:
                    prev = [self.load(hf, j, rs)]
                else:
                    prev = [] if self.init is None else [(1, self.init(hf, j, rs))]
                c, v = _signed_sum(prev + [(c, p)])
                again = any(m > n and self.unit[m] == self.unit[n] for m in uses)
                if (self.unit[n] < self.unit[self.last[j]] and not again) or (not prev and len(gamma) == 1):
                    acc_s[self.slot(hf, j) + (rs,)] = v
                    v = None
                self.acc[hf, j, rs.start] = (c, v)
            for j in sorted({j for _, _, j in gamma}):
                if self.last[j] == n:
                    for hf in range(2):
                        c, v = self.load(hf, j, rs)
                        self.done(hf, j, v if c > 0 else -v, rs)
            return p

    def layernorm_tasks(src, dst):
        def task(hf, g):
            y = _layernorm(src(hf, g))
            for t in range(ND):
                dst[hf, t, g:g + 8] = y[:, 128 * t:128 * t + 128]
            return [y[:, 0:128]]
        return [partial(task, hf, g) for g in range(0, QB, 8) for hf in range(2)]

    def ln1_tasks(i, dst):
        def src(hf, g):
            return x_s[rows(i, hf * QB + g // 16 * 16, 16), :].astype(F32)[g % 16:g % 16 + 8]
        return layernorm_tasks(src, dst)

    def advance_tasks():
        def task(hf, t, g):
            v = xnext_s[hf, t, g:g + 16]
            xn_s[hf, t, g:g + 16] = v
            return _split(v)
        return [partial(task, hf, t, g) for hf in range(2) for t in range(ND) for g in range(0, QB, 16)]

    def kq_ops(i, prods=None):
        def done(hf, j, val, rs):
            if j >= ND:
                q_s[first(i), hf, j - ND] = (val * QSCALE).astype(BF16)
            else:
                k_s[first(i), hf, j] = val.astype(BF16)
        return Matmul("kq", xnext_s if first(i) else xn_s, done, prods=prods).ops()

    def v_ops(i, prods=None):
        def done(hf, j, val, rs):
            v_s[first(i), hf, j] = val
        return Matmul("v", xnext_s if first(i) else xn_s, done, prods=prods).ops()

    def ring(i, b):
        return (2 * i + b) % RING if isinstance(i, int) else (2 * i + b) & (RING - 1)

    def key_blocks(i, b):
        return min(2 * i + b + 1, 3) if isinstance(i, int) else 3

    def tiles(i, g):
        if g >= H // 2:
            return []
        if first(i):
            return [(g % 2, 4 * (g // 2) + j) for j in range(4)]
        return [(b, h) for b in range(2) for h in (2 * g, 2 * g + 1)]

    def query_group():
        return sum((lane8 >= c).astype(I32) for c in CUTS[1:])

    def init_query_masks():
        qt_s[...] = jnp.zeros(qt_s.shape, U32)
        for j in range(32):
            slot_of_row = (((sub8 + 2 * j) & 63) * 13) >> 7
            qmask_s[j] = jnp.where(query_group() == slot_of_row, jnp.uint32(0xFFFFFFFF), jnp.uint32(0))

    def relayout(i, b, h, dep):
        def gate(v):
            vs = _split(v)
            return v if dep is None else _cat([after(dep, vs[0])] + vs[1:])

        if h == 0:
            for t in range(ND):
                q = _unpack(gate(q_s.bitcast(U32)[first(i), b, t]))
                qt_s[b, pl.ds(8 + 64 * t, 64), :] = pltpu.bitcast(q.T, U32)
            for t in range(ND):
                vt_s[ring(i, b), pl.ds(128 * t, 128), :] = gate(v_s[first(i), b, t]).T
        f0 = DH * h
        t0, t1 = f0 // 128, (f0 + DH - 1) // 128
        d = (lane8 - f0 % 128) & 127
        idx = (f0 % 128 + d - DH * ((d * 205) >> 12)) & 127
        ku = k_s.bitcast(U32)
        for g in range(0, QB // 2, 8):
            src = ku[first(i), b, t1, pl.ds(g, 8), :]
            if t0 != t1:
                src = jnp.where(lane8 >= 64, ku[first(i), b, t0, pl.ds(g, 8), :], src)
            krep_s[ring(i, b), h, pl.ds(g, 8), :] = jnp.take_along_axis(gate(src), idx, axis=1)

    def score_dots(i, b, h, pull):
        n = key_blocks(i, b)
        p0 = DH * h // 2
        parts = []
        for w in range(8):
            t = (8 * w - p0) % 64
            offs = [8 + p0 + (t + r) % 64 % 10 - r for r in range(8) if (t + r) % 64 < 60]
            v = qt_s[b, offs[0]:offs[0] + 8, :]
            if offs[-1] != offs[0]:
                cut = next(r for r in range(1, 8) if (t + r) % 64 % 10 == 0 and (t + r) % 64 < 60)
                v = jnp.where(sub8 < cut, v, qt_s[b, offs[-1]:offs[-1] + 8, :])
            parts.append(v & qmask_s[t // 2])
        w = _unpack(_cat(parts))
        kb = [krep_s[ring(i, b + 1 - n + j), h] for j in range(n)]
        if n < 3:
            return [lambda: _dot(_unpack(pull(_cat(kb))), w)]
        d = (lane8 - DH * h) & 127
        ka, kc = _split(kb[0]), _split(kb[2])
        merged = []
        for g in range(7):
            a0, a1 = [sum(r >= c for c in CUTS) for r in (16 * g, 16 * g + 8)]
            edge = DH * a0 if a0 == a1 else jnp.where(sub8 < 4, DH * a0, DH * a1)
            merged.append(jnp.where(d >= edge, kc[g], ka[g]))
        x0 = jnp.where(d >= 5 * DH, kc[7], jnp.where(d >= 4 * DH, kc[6], jnp.where(d >= 2 * DH, kc[3], kc[0])))
        x1 = jnp.where(d >= 2 * DH, kc[4], kc[1])
        x2 = jnp.where(d >= 2 * DH, kc[5], kc[2])
        x0, x1, x2 = [_split(_unpack(v).astype(F32)) for v in (x0, x1, x2)]
        odd = ((d >= DH) & (d < 2 * DH)) | ((d >= 3 * DH) & (d < 4 * DH))
        extra = [jnp.where(odd, x1[1], x0[0]), jnp.where(odd, x2[0], x0[1]), jnp.where(odd, x2[1], x1[0])]
        return [lambda: _dot(_cat(extra), w), lambda: _dot(_unpack(pull(_cat(merged + [ka[7], kb[1]]))), w)]

    def softmax_tasks(i, b, s, buf):
        n = key_blocks(i, b)
        rel = lane8 - sub8
        s = _split(s)
        if n == 3:
            vis = []
            for g in range(16):
                a = sum(8 * g >= c for c in CUTS) - 1
                causal = jnp.where(query_group() == a, rel, -1) >= 8 * g
                vis.append(jnp.where(causal, s[g - CUTS[a] // 8], s[3 + g]))
            vis += s[19:]
        else:
            vis = [jnp.where(rel >= 8 * g, s[16 * (n - 1) + g], -1e30) for g in range(16)] + s[:16 * (n - 1)]
        m = jnp.broadcast_to(jnp.max(functools.reduce(jnp.maximum, vis), axis=0, keepdims=True), (8, 128))
        s_s[buf, 0:8 * len(vis)] = _cat(vis)

        def task(r, dep):
            mr = m if dep is None else after(dep, m)
            p_s[buf, r:r + 16] = _cat([jnp.exp2(v - mr) for v in _split(s_s[buf, r:r + 16])]).astype(BF16)
        return [partial(task, r) for r in range(0, 8 * len(vis), 16)]

    def weighted_values(i, b, h, buf):
        n = key_blocks(i, b)
        ps = [p_s.bitcast(U32)[buf, 64 * j:64 * j + 64] for j in range(min(n, 2))][::-1]
        if n == 3:
            r = lax.broadcasted_iota(I32, (QB // 2, QB), 0) * 2
            c = lax.broadcasted_iota(I32, (QB // 2, QB), 1)
            causal = (jnp.where(r <= c, jnp.uint32(0xFFFF), jnp.uint32(0))
                      | jnp.where(r + 1 <= c, jnp.uint32(0xFFFF0000), jnp.uint32(0)))
            pc = ps[1] & causal
            ps = [ps[1] ^ pc, ps[0], pc]
        r0 = DH * h // 8 * 8
        o = None
        for j in range(n):
            vs = [vt_s[ring(i, b + 1 - n + j), r0 + g:r0 + g + 8, :] for g in (0, 8, 16)]
            if h % 2 == 0:
                vs[2] = jnp.where(sub8 >= 4, 1.0, vs[2])
            else:
                vs[0] = jnp.where(sub8 < 4, 1.0, vs[0])
            part = _dot(_cat(vs), _unpack(ps[j]))
            o = part if o is None else o + part
        return o

    def normalize(h, o):
        total = jnp.broadcast_to(o[23:24] if h % 2 == 0 else o[0:1], (8, 128))
        inv = pl.reciprocal(total, approx=True)
        inv = inv * (2.0 - total * inv)
        return [v * inv for v in _split(o)]

    def transpose_output(i, b, t, dep=None):
        vs = _split(ot_s[b, 128 * t:128 * t + 128, :])
        val = _cat(vs if dep is None else [after(dep, vs[0])] + vs[1:]).T
        o_s[first(i), b, t] = val
        return [val[QB - 8:]]

    def o_ops(i, prods=None):
        def init(hf, j, rs):
            return x_s[rows(i, hf * QB + rs.start, rs.stop - rs.start), 128 * j:128 * j + 128].astype(F32)

        def done(hf, j, val, rs):
            h_s[hf, rs, 128 * j:128 * j + 128] = val
        return Matmul("o", o_s.at[first(i)], done, init, prods).ops()

    def ln2_tasks():
        return layernorm_tasks(lambda hf, g: h_s[hf, g:g + 8, :], hn_s)

    def ffn_ops(i):
        def done1(hf, j, val, rs):
            f_s[hf, j, rs] = jnp.maximum(val, 0.0)

        def done2(hf, j, val, rs):
            out_s[rows(i, hf * QB, QB), 128 * j:128 * j + 128] = val.astype(out_s.dtype)

        f1 = Matmul("f1", hn_s, done1).ops()
        f2 = Matmul("f2", f_s, done2, lambda hf, j, rs: h_s[hf, rs, 128 * j:128 * j + 128]).ops()
        n1 = len(f1)
        return [(f1 if j < n1 else f2).pop(0) for j in ORDER["ffn"]]

    def units(ops):
        for n, (mm, m) in enumerate(ops):
            mm.unit[m] = n // 4
        return [("dense", ops[j:j + 4], slice(0, QB)) for j in range(0, len(ops), 4)]

    def halves(us):
        return [("dense", u, slice(r, r + QB // 2)) for r in (0, QB // 2) for _, u, _ in us]

    def with_attention(i, parts):
        seq = [("scores", i, 0)]
        for g in range(H // 2):
            seq += ([("scores", i, g + 1)] if g + 1 < H // 2 else []) + [("values", i, g)]
        plan = []
        for dense, n in parts:
            done = 0
            for j in range(n):
                plan.append(seq.pop(0))
                while done < len(dense) * (j + 1) / n - 0.5:
                    plan.append(dense[done])
                    done += 1
            plan += dense[done:]
        assert not seq
        return plan

    def beats(e):
        if e[0] == "dense":
            return (e[2].stop - e[2].start) // 8
        if e[0] == "call":
            return 0
        n = key_blocks(e[1], tiles(e[1], e[2])[0][0])
        return 3 * n if e[0] == "values" else (16, 32, 35)[n - 1]

    class Plan:
        def __init__(self, steps):
            self.steps = steps
            self.start = [0]
            for e in steps:
                self.start.append(self.start[-1] + beats(e))
            self.due = []

        def times(self, kind, uses=None):
            return [t for e, t in zip(self.steps, self.start)
                    if e[0] == kind and (uses is None or any(uses(mm.name, mm.prods[n][1]) for mm, n in e[1]))]

        def spread(self, tasks, t0, t1):
            self.due += [(t0 + (t1 - t0) * n / len(tasks), fn) for n, fn in enumerate(tasks)]

        def sum_weights(self, name, t0, t1):
            def needed(group):
                ts = self.times("dense", lambda n, beta: n == name and beta in group[1])
                return min([t for t in ts if t > t0] + [t1 + 12]) - 12

            groups = sorted(weight_sum_tasks(name), key=needed)
            t = t1
            for group in groups[::-1]:
                t = min(t, needed(group))
                dt = (t1 - t0) * group[0] / sum(g[0] for g in groups)
                self.spread(group[2], max(t - dt, t0), max(t, t0))
                t -= dt

        def pull(self, n):
            t0, end = self.start[n], self.times("dense")[-1]
            t1 = self.start[n + 2 if [e[0] for e in self.steps[n + 1:n + 2]] == ["values"] else n + 1]
            now = sorted((w for w in self.due if min(w[0], end) < t1), key=lambda w: w[0])
            self.due = [w for w in self.due if min(w[0], end) >= t1]
            deps = [(min(max((t - t0) / (t1 - t0), 0), 0.999), dep) for t, fn in now for dep in fn()]

            def apply(lhs):
                vs = _split(lhs)
                for g in range(len(vs)):
                    ds = [dep for t, dep in deps if int(t * len(vs)) == g]
                    if ds:
                        vs[g] = after(functools.reduce(jnp.maximum, ds), vs[g])
                return _cat(vs)
            return apply

        def push(self, val):
            for dep in _split(val):
                if self.skip > 0:
                    self.skip -= 1
                    continue
                self.credit += self.rate
                while self.queue and self.credit >= 1:
                    self.credit -= 1
                    self.queue.pop(0)[1](dep)

        def scores(self, n, i, g):
            pull = self.pull(n)
            for ahead in ([g + 1] if g > 0 else [0, 1]):
                for b, h in sorted(tiles(i, ahead), key=lambda bh: bh[::-1]):
                    relayout(i, b, h, self.mark)
            dots = [score_dots(i, b, h, pull if j == 3 else (lambda v: v)) for j, (b, h) in enumerate(tiles(i, g))]
            dots = [_cat(ds) for ds in zip(*[[fn() for fn in fns] for fns in zip(*dots)])]
            tasks = []
            for j, (b, h) in enumerate(tiles(i, g)):
                if j == 3:
                    self.push(dots[j])
                tasks += softmax_tasks(i, b, dots[j], (4 * g + j) % NBUF)
            self.mark = dots[3][0:8]
            self.queue += [(g, fn) for fn in tasks]
            end, window = self.steps.index(("values", i, g)), 0
            for m in range(n + 1, end):
                if self.steps[m][0] != "values":
                    window += max(min(beats(self.steps[m]), self.start[end] - 16 - self.start[m]), 0)
                if self.steps[m][0] == "scores":
                    break
            self.skip, self.credit = 3, 0.0
            self.rate = len(self.queue) / max((window - self.skip) * 0.8, 1)

        def values(self, n, i, g):
            while self.queue and self.queue[0][0] <= g:
                self.queue.pop(0)[1](None)
            ts = tiles(i, g)
            outs = [weighted_values(i, b, h, (4 * g + j) % NBUF) for j, (b, h) in enumerate(ts)]
            for j in (0, 2):
                b, h = ts[j]
                lo, hi = normalize(h, outs[j]), normalize(h + 1, outs[j + 1])
                ot_s[b, DH * h:DH * (h + 2), :] = _cat(lo[:2] + [jnp.where(sub8 < 4, lo[2], hi[0])] + hi[1:])
                t = DH * (h + 2) // 128 - 1
                if first(i) and t >= 0 and DH * h < 128 * (t + 1):
                    self.due.append((self.start[n] + 80, partial(lambda v: v, transpose_output(i, b, t))))
            if not first(i) and g == H // 2 - 1:
                self.spread([partial(transpose_output, i, b, t, self.mark) for t in range(ND) for b in range(2)],
                            self.start[n] + 30, self.start[n] + 110)

        def run(self):
            self.queue, self.rate, self.credit, self.skip, self.mark = [], 0.0, 0.0, 0, None
            for n, e in enumerate(self.steps):
                if e[0] == "call":
                    e[1]()
                elif e[0] == "dense":
                    pull = self.pull(n)
                    for j, (mm, m) in enumerate(e[1]):
                        p = mm.run(m, e[2], pull if j == 0 else (lambda v: v))
                        if j == 0:
                            self.push(p)
                elif e[0] == "scores":
                    self.scores(n, e[1], e[2])
                else:
                    self.values(n, e[1], e[2])
            assert not self.due and not self.queue

    def prologue():
        for copies in (x_copies(0), x_copies(1), w_copies(0), w_copies(1), w_copies(2), w_copies(3), w_copies(4),
                       w_copies(5) + w_copies(6), w_copies(7), x_copies(2), x_copies(3)):
            for c in copies:
                c.start()
            pl.semaphore_signal(sem_order)
            pl.semaphore_wait(sem_order)
        init_query_masks()
        for i, dst in enumerate((xnext_s, xn_s)):
            wait(x_copies(i))
            for fn in ln1_tasks(i, dst):
                fn()
        wait(w_copies(0))
        v0, v1 = v_ops(0, _scheme(*SHAPES["v"])), v_ops(1, _scheme(*SHAPES["v"]))
        kq0, kq1 = units(kq_ops(0, _scheme(*SHAPES["kq"]))), units(kq_ops(1))
        o0 = units(o_ops(0, sorted(SCHEMES["o"], key=lambda p: len(p[1]) > 1)))
        f0 = units(ffn_ops(0))
        a0 = with_attention(0, [(kq1[:-7], 29), (kq1[-7:-4], 2), (kq1[-4:], 1)])
        a1 = with_attention(1, [(o0, 2), ([], 3), (f0[:-8], 26), (f0[-8:], 1)])
        plan = Plan(units(v0[:10] + v1[:10]) + [("call", partial(wait, w_copies(1)))]
                    + units(v0[10:30] + v1[10:30]) + [("call", partial(wait, w_copies(2)))]
                    + units(v0[30:] + v1[30:]) + [("call", partial(wait, w_copies(3)))]
                    + kq0[:12] + [("call", partial(wait, w_copies(4)))] + kq0[12:]
                    + a0[:35] + [("call", partial(wait, w_copies(5) + w_copies(6)))] + a0[35:]
                    + a1[:24] + [("call", partial(wait, w_copies(7) + x_copies(2)))] + a1[24:])
        arrived, end = plan.times("call"), plan.start[-1]
        o_at, f1_at = [plan.times("dense", lambda n, _: n == name) for name in ("o", "f1")]
        plan.sum_weights("v", arrived[1], arrived[3])
        plan.sum_weights("kq", arrived[3], arrived[3] + 16 * 13)
        plan.sum_weights("f1", arrived[4] + 16, f1_at[-1])
        plan.sum_weights("f2", arrived[5] + 16, end - 30)
        plan.sum_weights("o", arrived[4] + 16, o_at[-1])
        plan.spread(ln2_tasks(), f1_at[0] - 30, f1_at[0])
        plan.spread(ln1_tasks(2, xn_s), end - 150, end - 10)
        plan.run()
        wait(x_copies(3))

    def step(i, carry):
        proj = units(o_ops(i - 1) + kq_ops(i) + v_ops(i))
        ffn = units(ffn_ops(i - 1))
        plan = Plan(proj[:2] + [("call", out_copy(i - 2).start)] + proj[2:]
                    + with_attention(i, [(ffn[:-8], 31), (ffn[-8:], 1)]))
        t0, t1 = 16 * len(proj), plan.start[-1]
        plan.spread(ln2_tasks(), 236, 600)
        plan.spread(ln1_tasks(jnp.minimum(i + 1, NSTEP - 1), xnext_s), 420, t0)
        plan.spread(advance_tasks(), t0 + 0.1 * (t1 - t0), t0 + 0.9 * (t1 - t0))
        plan.run()
        return carry

    def epilogue():
        wait([out_copy(i) for i in range(NSTEP - 2)])
        out_copy(NSTEP - 2).start()
        proj, ffn = units(o_ops(NSTEP - 1)), units(ffn_ops(NSTEP - 1))
        f2 = ffn[-1][1][-1][0]
        steps = halves(proj) + halves(ffn[:8])
        for n in range(8, len(ffn)):
            steps += [ffn[n]] + [("call", last_out_copy(j).start) for j in range(ND)
                                 if min(f2.unit[f2.last[j]] + 2, len(ffn) - 1) == n]
        plan, tasks, t = Plan(steps), ln2_tasks(), 16 * len(proj)
        plan.spread(tasks[:16], t - 16, t)
        plan.spread(tasks[16:], t + 48, t + 64)
        plan.run()
        wait([out_copy(NSTEP - 2)] + [last_out_copy(j) for j in range(ND)])

    prologue()
    lax.fori_loop(2, NSTEP, step, 0)
    epilogue()


@jax.jit
def pallas_sequential_preLN__sliding_block__dense_activation_relu__prompt_kernel(
    A_x: jax.Array,
    A_wqkv: jax.Array,
    A_wo: jax.Array,
    B_x: jax.Array,
    B_w1: jax.Array,
    B_w2: jax.Array,
):
    del B_x
    any_spec = pl.BlockSpec(memory_space=pl.ANY)
    out = pl.pallas_call(
        _kernel,
        in_specs=[any_spec] * 5,
        out_specs=any_spec,
        out_shape=jax.ShapeDtypeStruct((S, D), A_x.dtype),
        scratch_shapes=[
            pltpu.VMEM((S, D), BF16),
            pltpu.VMEM((S, D), BF16),
            pltpu.VMEM((3 * ND, D, 128), BF16),
            pltpu.VMEM((ND, D, 128), BF16),
            pltpu.VMEM((NF, D, 128), BF16),
            pltpu.VMEM((ND, DFF, 128), BF16),
            pltpu.VMEM((len(WEIGHT_SUMS), 128, 128), BF16),
            pltpu.VMEM((2, ND, QB, 128), F32),
            pltpu.VMEM((2, ND, QB, 128), F32),
            pltpu.VMEM((2, 2, ND, QB, 128), BF16),
            pltpu.VMEM((2, 2, ND, QB, 128), BF16),
            pltpu.VMEM((2, 2, ND, QB, 128), F32),
            pltpu.VMEM((RING, H, QB // 2, 128), U32),
            pltpu.VMEM((2, D // 2 + 16, 128), U32),
            pltpu.VMEM((32, 8, 128), U32),
            pltpu.VMEM((RING, D, 128), F32),
            pltpu.VMEM((NBUF, 2 * QB, 128), F32),
            pltpu.VMEM((NBUF, 2 * QB, 128), BF16),
            pltpu.VMEM((2, D, 128), F32),
            pltpu.VMEM((2, 2, ND, QB, 128), F32),
            pltpu.VMEM((2, QB, D), F32),
            pltpu.VMEM((2, ND, QB, 128), F32),
            pltpu.VMEM((2, NF, QB, 128), F32),
            pltpu.VMEM((2, NF + ND, QB, 128), F32),
            pltpu.SemaphoreType.DMA((4,)),
            pltpu.SemaphoreType.DMA((8,)),
            pltpu.SemaphoreType.DMA((NSTEP,)),
            pltpu.SemaphoreType.REGULAR,
        ],
        compiler_params=pltpu.CompilerParams(vmem_limit_bytes=100 * 1024 * 1024),
        name="fused_block",
    )(A_x.reshape(S, D), A_wqkv, A_wo, B_w1, B_w2)
    return out.reshape(A_x.shape)
```

```python
import functools

import jax
import jax.experimental.pallas as pl
import jax.experimental.pallas.tpu as pltpu
import jax.numpy as jnp
import numpy as np
from jax import lax

S, D, H, DH, DFF = 2048, 640, 32, 20, 1536
QB = 128
T = 2 * QB
NSTEP = S // T
ND, NF = D // 128, DFF // 128
RING = 4
CUTS = (0, 24, 48, 72, 96, 112)
NBUF = 16
EPS = 1e-5
QSCALE = DH ** -0.5 * 1.4426950408889634
BF16, F32, U32, I32 = jnp.bfloat16, jnp.float32, jnp.uint32, jnp.int32
partial = functools.partial


def _scheme(nk, nn, diag=(), pairs=()):
    pts = np.array([[1, 0], [0, 1], [-1, -1]])
    perp = np.array([[0, -1], [1, 0], [-1, 1]])
    ek, en = np.eye(nk, dtype=int), np.eye(nn, dtype=int)
    els, prods, covered = [], [], np.zeros((nk, nn), bool)
    for i, j, m in diag:
        s, t = (m + 1) % 3, (m + 2) % 3
        els.append((ek[i], en[j], m))
        prods += [(np.outer(pts[s], ek[i]), np.outer(perp[t], en[j])),
                  (np.outer(pts[t], ek[i]), np.outer(perp[s], en[j]))]
        covered[i, j] = True
    for e, e2 in pairs:
        (a, c, t), (a2, c2, s) = els[e], els[e2]
        prods += [(np.outer(pts[s], a + a2), np.outer(perp[t], c + c2)),
                  (np.outer(pts[t], a + a2), np.outer(perp[s], c + c2)),
                  (np.outer(pts[s], a) - np.outer(pts[t], a2), np.outer(perp[s], c) - np.outer(perp[t], c2))]
        els.append((a + a2, c + c2, 3 - s - t))
        covered |= (np.outer(a, c2) + np.outer(a2, c)) != 0
    for j in range(nn):
        for i in range(nk):
            if not covered[i, j]:
                prods += [(np.outer(pts[hf], ek[i]), np.outer(pts[hf], en[j])) for hf in range(2)]
    lhs = np.stack([np.kron(a.ravel(), c.ravel()) for a, c in prods], axis=1)
    rhs = np.einsum("hg,ik,jl->higjkl", np.eye(2, dtype=int), ek, en).reshape(lhs.shape[0], -1)
    w = np.rint(np.linalg.lstsq(lhs.astype(float), rhs.astype(float), rcond=None)[0]).astype(int)
    assert np.array_equal(lhs @ w, rhs) and max(np.abs(lhs).max(), np.abs(w).max()) == 1

    def terms(m, sign):
        return tuple((int(sign * m[r, c]), int(r), int(c)) for r, c in zip(*np.nonzero(m)))

    out = []
    for (a, c), b in zip(prods, w.reshape(-1, nk, nn)):
        sa, sb = a[a != 0][0], b[b != 0][0]
        out.append((terms(a, sa), terms(b, sb), terms(c, sa * sb)))
    return out


ORDER = dict(
    kq=[43, 55, 41, 18, 38, 68, 32, 77, 39, 36, 27, 24, 44, 56, 65, 53, 40, 26, 16, 28, 33, 34, 42, 3, 54, 21, 48,
        30, 22, 25, 20, 23, 0, 29, 31, 1, 71, 73, 8, 59, 51, 50, 5, 52, 66, 19, 67, 7, 45, 46, 58, 57, 4, 47, 49,
        12, 78, 9, 79, 17, 37, 35, 14, 2, 72, 61, 60, 13, 11, 10, 70, 69, 62, 63, 64, 6, 74, 75, 15, 76],
    v=[25, 35, 9, 16, 20, 23, 14, 11, 17, 18, 34, 36, 3, 27, 26, 2, 32, 33, 31, 37, 12, 0, 4, 10, 22, 24, 19, 21,
       13, 6, 1, 15, 38, 8, 7, 39, 30, 5, 29, 28],
    o=[0, 36, 17, 34, 11, 12, 1, 4, 38, 31, 28, 8, 15, 14, 24, 23, 19, 22, 10, 13, 37, 29, 39, 30, 5, 20, 21, 3, 9,
       16, 35, 18, 33, 6, 7, 32, 26, 2, 25, 27],
    f2=[23, 20, 35, 47, 26, 56, 44, 50, 65, 77, 68, 29, 18, 71, 41, 43, 48, 39, 51, 60, 57, 45, 24, 63, 22, 59, 28,
        12, 1, 27, 25, 64, 10, 49, 46, 32, 21, 69, 72, 42, 76, 14, 62, 79, 75, 52, 54, 5, 9, 70, 78, 58, 30, 19, 31,
        8, 15, 37, 3, 36, 53, 55, 74, 4, 33, 34, 0, 11, 73, 61, 66, 67, 40, 2, 13, 38, 7, 6, 16, 17],
    g1=[24, 22, 33, 32, 20, 21, 5, 4, 7, 6, 28, 29, 14, 3, 15, 2, 25, 8, 27, 26, 18, 16, 30, 31, 0, 1, 12, 11, 23, 9,
        10, 17, 19, 13],
    g2=[30, 31, 28, 29, 10, 21, 4, 20, 11, 1, 0, 12, 19, 25, 7, 13, 17, 16, 8, 18, 24, 5, 22, 23, 15, 3, 14, 2, 26, 6,
        27, 9, 32, 33])
ORDER["f1"] = ORDER["kq"]


def _schemes():
    d10 = [(j % 5, j, j // 5) for j in range(10)]
    p10 = [(a, b) for a in range(5) for b in range(5, 10) if a != b - 5]
    d4 = [(0, 0, 0), (0, 4, 1), (1, 1, 1), (2, 2, 0), (3, 3, 2)]
    p4 = [(0, 2), (1, 3), (1, 4), (2, 3), (2, 4), (3, 4)]
    d5 = [(i, i, (0, 0, 1, 1, 2)[i]) for i in range(5)]
    p5 = [(0, 2), (0, 3), (0, 4), (1, 2), (1, 3), (1, 4), (2, 4), (3, 4), (7, 1), (11, 3)]
    kq, sq = _scheme(5, 10, d10, p10), _scheme(5, 5, d5, p5)
    f2 = _scheme(10, 5, [(j, i, m) for i, j, m in d10], p10)

    def flip(terms, off=0):
        return tuple((c, col, row + off) for c, row, col in terms)

    def signed(a, b, c):
        sa, sb = a[0][0], b[0][0]
        return tuple(tuple((s * e, r, k) for e, r, k in t) for s, t in ((sa, a), (sb, b), (sa * sb, c)))

    rest = _scheme(4, 5, d4, p4)
    out = dict(kq=kq, v=sq, o=sq, f1=kq, f2=f2, g1=[signed(b, flip(c, 10), flip(a, 10)) for a, b, c in rest],
               g2=[signed(flip(a, 10), tuple((e, r + 10, k) for e, r, k in c), b) for a, b, c in rest])
    assert all(sorted(ORDER[n]) == list(range(len(p))) for n, p in out.items())
    return {n: [p[j] for j in ORDER[n]] for n, p in out.items()}


SCHEMES = _schemes()
WEIGHT_SUMS = {}
for _name, _prods in SCHEMES.items():
    for _, _beta, _ in _prods:
        if len(_beta) > 1:
            WEIGHT_SUMS.setdefault((_name, _beta), len(WEIGHT_SUMS))


def _dot(a, b):
    return lax.dot_general(a, b, (((1,), (0,)), ((), ())), preferred_element_type=F32)


def _layernorm(x):
    c = x - jnp.mean(x, axis=-1, keepdims=True)
    return c * lax.rsqrt(jnp.mean(c * c, axis=-1, keepdims=True) + EPS)


def _unpack(x):
    return pltpu.bitcast(x, BF16)


def _split(x):
    return [x[g:g + 8] for g in range(0, x.shape[0], 8)]


def _cat(xs):
    return xs[0] if len(xs) == 1 else jnp.concatenate(xs, axis=0)


def _signed_sum(terms):
    first = next((n for n, (c, _) in enumerate(terms) if c > 0), None)
    sign = -1 if first is None else 1
    acc = terms[first or 0][1]
    for n, (c, v) in enumerate(terms):
        if n != (first or 0):
            acc = acc + v if c * sign > 0 else acc - v
    return sign, acc


def _kernel(x_hbm, wqkv_hbm, wo_hbm, w1_hbm, w2_hbm, out_hbm,
            x_s, out_s, wqkv_s, wo_s, w1_s, w2_s, wsum_s, xn_s, xnext_s, k_s, q_s, v_s, krep_s, qt_s, qmask_s, vt_s,
            s_s, p_s, ot_s, o_s, h_s, hn_s, f_s, acc_s, sem_x, sem_w, sem_o, sem_order):
    sub8 = lax.broadcasted_iota(I32, (8, 128), 0)
    lane8 = lax.broadcasted_iota(I32, (8, 128), 1)

    memo = {}

    def once(fn):
        def cached(*args):
            if (fn, args) not in memo:
                memo[fn, args] = fn(*args)
            return memo[fn, args]
        return cached

    def rows(i, off=0, n=T):
        r = i * T + off
        return pl.ds(r if isinstance(r, int) else pl.multiple_of(r, 16), n)

    def first(i):
        return int(isinstance(i, int) and i == 0)

    @once
    def never():
        return qmask_s[0] == 1

    def after(dep, val):
        return lax.select(never(), dep if dep.dtype == val.dtype else pltpu.bitcast(dep, val.dtype), val)

    def x_copies(j):
        r = pl.ds(j * T, T if j < 3 else S - 3 * T)
        return [pltpu.make_async_copy(x_hbm.at[r], x_s.at[r], sem_x.at[j])]

    def w_copies(j):
        src, dst, t0, t1 = ((wqkv_hbm, wqkv_s, 2 * ND, 2 * ND + 1), (wqkv_hbm, wqkv_s, 2 * ND + 1, 2 * ND + 3),
                            (wqkv_hbm, wqkv_s, 2 * ND + 3, 3 * ND), (wqkv_hbm, wqkv_s, ND, 2 * ND),
                            (wqkv_hbm, wqkv_s, 0, ND), (wo_hbm, wo_s, 0, ND), (w1_hbm, w1_s, 0, NF),
                            (w2_hbm, w2_s, 0, ND))[j]
        return [pltpu.make_async_copy(src.at[:, pl.ds(128 * t, 128)], dst.at[t], sem_w.at[j]) for t in range(t0, t1)]

    def out_copy(i):
        return pltpu.make_async_copy(out_s.at[rows(i)], out_hbm.at[rows(i)], sem_o.at[i])

    def last_out_copy(j):
        win = (rows(NSTEP - 1), pl.ds(128 * j, 128))
        return pltpu.make_async_copy(out_s.at[win], out_hbm.at[win], sem_o.at[NSTEP - 1])

    def wait(copies):
        for c in copies:
            c.wait()

    def weight(name, i, j, r0=0, n=128):
        if name == "kq":
            ref, j = wqkv_s, (j + ND) % (2 * ND)
        elif name == "v":
            ref, j = wqkv_s, j + 2 * ND
        else:
            ref = dict(o=wo_s, f1=w1_s, g1=w1_s, f2=w2_s, g2=w2_s)[name]
        return _unpack(ref.bitcast(U32)[j, pl.ds((128 * i + r0) // 2, n // 2), :])

    def weight_sum_tasks(name):
        groups = []
        for beta in sorted((b for n, b in WEIGHT_SUMS if n == name), key=lambda b: -len(b)):
            src = {t[1:] for t in beta}
            best = max(groups, key=lambda g: len(g[0] & src), default=None)
            if best is not None and best[0] & src and len(best[0] | src) <= 9:
                best[0].update(src)
                best[1].append(beta)
            else:
                groups.append((src, [beta]))

        def task(beta, r0):
            _, w = _signed_sum([(c, weight(name, i, j, r0, 16).astype(F32)) for c, i, j in beta])
            wsum_s[WEIGHT_SUMS[name, beta], r0:r0 + 16] = w.astype(BF16)
            return _split(w)

        return [(len(src) + sum(map(len, betas)), betas,
                 [partial(task, beta, r0) for r0 in range(0, 128, 16) for beta in betas]) for src, betas in groups]

    class Matmul:
        def __init__(self, name, a_ref, done, init=None, prods=None):
            self.name, self.a_ref, self.done, self.init = name, a_ref, done, init
            self.prods = prods or SCHEMES[name]
            self.unit = [0] * len(self.prods)
            self.last = {j: n for n, (_, _, gamma) in enumerate(self.prods) for _, _, j in gamma}
            self.acc = {}
            self.parts = 4 if name in ("g1", "g2") else 2

        def place(self, part, rs):
            hf, r0 = divmod(part * (T // self.parts), QB)
            return hf, slice(r0 + rs.start, r0 + rs.stop)

        def ops(self):
            return [(self, n) for n in range(len(self.prods))]

        def slot(self, part, j, rs):
            hf, rs = self.place(part, rs)
            return hf, j + (NF if self.name in ("f2", "g2") else 0), rs

        def load(self, hf, j, rs):
            c, v = self.acc.get((hf, j, rs.start)) or self.acc[hf, j, 0]
            return c, (acc_s[self.slot(hf, j, rs)] if v is None else v)

        def run(self, n, rs, pull):
            alpha, beta, gamma = self.prods[n]
            _, lhs = _signed_sum([(c, self.a_ref[self.place(hf, rs)[0], i, self.place(hf, rs)[1]]) for c, hf, i in alpha])
            if len(beta) == 1:
                w = weight(self.name, *beta[0][1:])
            else:
                w = _unpack(wsum_s.bitcast(U32)[WEIGHT_SUMS[self.name, beta]])
            p = _dot(pull(lhs), w)
            for c, hf, j in gamma:
                uses = [m for m, (_, _, g) in enumerate(self.prods) if any((hf, j) == t[1:] for t in g)]
                if uses[0] < n:
                    prev = [self.load(hf, j, rs)]
                else:
                    prev = [] if self.init is None else [(1, self.init(self.place(hf, rs)[0], j, self.place(hf, rs)[1]))]
                c, v = _signed_sum(prev + [(c, p)])
                again = any(m > n and self.unit[m] == self.unit[n] for m in uses)
                if (self.unit[n] < self.unit[self.last[j]] and not again) or (not prev and len(gamma) == 1):
                    acc_s[self.slot(hf, j, rs)] = v
                    v = None
                self.acc[hf, j, rs.start] = (c, v)
            for j in sorted({j for _, _, j in gamma}):
                if self.last[j] == n:
                    for hf in range(self.parts):
                        c, v = self.load(hf, j, rs)
                        self.done(self.place(hf, rs)[0], j, v if c > 0 else -v, self.place(hf, rs)[1])
            return p

    def layernorm_tasks(src, dst):
        def task(hf, g):
            y = _layernorm(src(hf, g))
            for t in range(ND):
                dst[hf, t, g:g + 8] = y[:, 128 * t:128 * t + 128]
            return [y[:, 0:128]]
        return [partial(task, hf, g) for g in range(0, QB, 8) for hf in range(2)]

    def ln1_tasks(i, dst):
        def src(hf, g):
            return x_s[rows(i, hf * QB + g // 16 * 16, 16), :].astype(F32)[g % 16:g % 16 + 8]
        return layernorm_tasks(src, dst)

    def advance_tasks():
        def task(hf, t, g):
            v = xnext_s[hf, t, g:g + 16]
            xn_s[hf, t, g:g + 16] = v
            return _split(v)
        return [partial(task, hf, t, g) for hf in range(2) for t in range(ND) for g in range(0, QB, 16)]

    def kq_ops(i, prods=None):
        def done(hf, j, val, rs):
            if j >= ND:
                q_s[first(i), hf, j - ND] = (val * QSCALE).astype(BF16)
            else:
                k_s[first(i), hf, j] = val.astype(BF16)
        return Matmul("kq", xnext_s if first(i) else xn_s, done, prods=prods).ops()

    def v_ops(i, prods=None):
        def done(hf, j, val, rs):
            v_s[first(i), hf, j] = val
        return Matmul("v", xnext_s if first(i) else xn_s, done, prods=prods).ops()

    def ring(i, b):
        return (2 * i + b) % RING if isinstance(i, int) else (2 * i + b) & (RING - 1)

    def key_blocks(i, b):
        return min(2 * i + b + 1, 3) if isinstance(i, int) else 3

    def tiles(i, g):
        if g >= H // 2:
            return []
        if first(i):
            return [(g % 2, 4 * (g // 2) + j) for j in range(4)]
        return [(b, h) for b in range(2) for h in (2 * g, 2 * g + 1)]

    @once
    def query_group():
        return sum((lane8 >= c).astype(I32) for c in CUTS[1:])

    def init_query_masks():
        qt_s[...] = jnp.zeros(qt_s.shape, U32)
        for j in range(32):
            slot_of_row = (((sub8 + 2 * j) & 63) * 13) >> 7
            qmask_s[j] = jnp.where(query_group() == slot_of_row, jnp.uint32(0xFFFFFFFF), jnp.uint32(0))

    def relayout(i, b, h, dep):
        def gate(v):
            vs = _split(v)
            return v if dep is None else _cat([after(dep, vs[0])] + vs[1:])

        if h == 0:
            for t in range(ND):
                q = _unpack(gate(q_s.bitcast(U32)[first(i), b, t]))
                qt_s[b, pl.ds(8 + 64 * t, 64), :] = pltpu.bitcast(q.T, U32)
            for t in range(ND):
                vt_s[ring(i, b), pl.ds(128 * t, 128), :] = gate(v_s[first(i), b, t]).T
        f0 = DH * h
        t0, t1 = f0 // 128, (f0 + DH - 1) // 128
        d = (lane8 - f0 % 128) & 127
        idx = (f0 % 128 + d - DH * ((d * 205) >> 12)) & 127
        ku = k_s.bitcast(U32)
        for g in range(0, QB // 2, 8):
            src = ku[first(i), b, t1, pl.ds(g, 8), :]
            if t0 != t1:
                src = jnp.where(lane8 >= 64, ku[first(i), b, t0, pl.ds(g, 8), :], src)
            krep_s[ring(i, b), h, pl.ds(g, 8), :] = jnp.take_along_axis(gate(src), idx, axis=1)

    def score_dots(i, b, h, pull):
        n = key_blocks(i, b)
        p0 = DH * h // 2
        parts = []
        for w in range(8):
            t = (8 * w - p0) % 64
            offs = [8 + p0 + (t + r) % 64 % 10 - r for r in range(8) if (t + r) % 64 < 60]
            v = qt_s[b, offs[0]:offs[0] + 8, :]
            if offs[-1] != offs[0]:
                cut = next(r for r in range(1, 8) if (t + r) % 64 % 10 == 0 and (t + r) % 64 < 60)
                v = jnp.where(sub8 < cut, v, qt_s[b, offs[-1]:offs[-1] + 8, :])
            parts.append(v & qmask_s[t // 2])
        w = _unpack(_cat(parts))
        kb = [krep_s[ring(i, b + 1 - n + j), h] for j in range(n)]
        if n < 3:
            return [lambda: _dot(_unpack(pull(_cat(kb))), w)]
        d = (lane8 - DH * h) & 127
        ka, kc = _split(kb[0]), _split(kb[2])
        merged = []
        for g in range(7):
            a0, a1 = [sum(r >= c for c in CUTS) for r in (16 * g, 16 * g + 8)]
            edge = DH * a0 if a0 == a1 else jnp.where(sub8 < 4, DH * a0, DH * a1)
            merged.append(jnp.where(d >= edge, kc[g], ka[g]))
        x0 = jnp.where(d >= 5 * DH, kc[7], jnp.where(d >= 4 * DH, kc[6], jnp.where(d >= 2 * DH, kc[3], kc[0])))
        x1 = jnp.where(d >= 2 * DH, kc[4], kc[1])
        x2 = jnp.where(d >= 2 * DH, kc[5], kc[2])
        x0, x1, x2 = [_split(_unpack(v).astype(F32)) for v in (x0, x1, x2)]
        odd = ((d >= DH) & (d < 2 * DH)) | ((d >= 3 * DH) & (d < 4 * DH))
        extra = [jnp.where(odd, x1[1], x0[0]), jnp.where(odd, x2[0], x0[1]), jnp.where(odd, x2[1], x1[0])]
        return [lambda: _dot(_cat(extra), w), lambda: _dot(_unpack(pull(_cat(merged + [ka[7], kb[1]]))), w)]

    @once
    def causal(g, group):
        rel = lane8 - sub8
        return (rel if group is None else jnp.where(query_group() == group, rel, -1)) >= 8 * g

    @once
    def causal_bits():
        r = lax.broadcasted_iota(I32, (QB // 2, QB), 0) * 2
        c = lax.broadcasted_iota(I32, (QB // 2, QB), 1)
        return (jnp.where(r <= c, jnp.uint32(0xFFFF), jnp.uint32(0))
                | jnp.where(r + 1 <= c, jnp.uint32(0xFFFF0000), jnp.uint32(0)))

    def softmax_tasks(i, b, s, buf):
        n = key_blocks(i, b)
        s = _split(s)
        if n == 3:
            vis = []
            for g in range(16):
                a = sum(8 * g >= c for c in CUTS) - 1
                vis.append(lax.select(causal(g, a), s[g - CUTS[a] // 8], s[3 + g]))
            vis += s[19:]
        else:
            vis = [jnp.where(causal(g, None), s[16 * (n - 1) + g], -1e30) for g in range(16)] + s[:16 * (n - 1)]
        m = jnp.broadcast_to(jnp.max(functools.reduce(jnp.maximum, vis), axis=0, keepdims=True), (8, 128))
        s_s[buf, 0:8 * len(vis)] = _cat(vis)

        def task(r, dep):
            mr = m if dep is None else after(dep, m)
            p_s[buf, r:r + 16] = _cat([jnp.exp2(v - mr) for v in _split(s_s[buf, r:r + 16])]).astype(BF16)
        return [partial(task, r) for r in range(0, 8 * len(vis), 16)]

    def weighted_values(i, b, h, buf):
        n = key_blocks(i, b)
        ps = [p_s.bitcast(U32)[buf, 64 * j:64 * j + 64] for j in range(min(n, 2))][::-1]
        if n == 3:
            pc = ps[1] & causal_bits()
            ps = [ps[1] ^ pc, ps[0], pc]
        r0 = DH * h // 8 * 8
        o = None
        for j in range(n):
            vs = [vt_s[ring(i, b + 1 - n + j), r0 + g:r0 + g + 8, :] for g in (0, 8, 16)]
            if h % 2 == 0:
                vs[2] = jnp.where(sub8 >= 4, 1.0, vs[2])
            else:
                vs[0] = jnp.where(sub8 < 4, 1.0, vs[0])
            part = _dot(_cat(vs), _unpack(ps[j]))
            o = part if o is None else o + part
        return o

    def normalize(h, o):
        total = jnp.broadcast_to(o[23:24] if h % 2 == 0 else o[0:1], (8, 128))
        inv = pl.reciprocal(total, approx=True)
        inv = inv * (2.0 - total * inv)
        return [v * inv for v in _split(o)]

    def transpose_output(i, b, t, dep=None):
        vs = _split(ot_s[b, 128 * t:128 * t + 128, :])
        val = _cat(vs if dep is None else [after(dep, vs[0])] + vs[1:]).T
        o_s[first(i), b, t] = val
        return [val[QB - 8:]]

    def o_ops(i, prods=None):
        def init(hf, j, rs):
            return x_s[rows(i, hf * QB + rs.start, rs.stop - rs.start), 128 * j:128 * j + 128].astype(F32)

        def done(hf, j, val, rs):
            h_s[hf, rs, 128 * j:128 * j + 128] = val
        return Matmul("o", o_s.at[first(i)], done, init, prods).ops()

    def ln2_tasks():
        return layernorm_tasks(lambda hf, g: h_s[hf, g:g + 8, :], hn_s)

    def ffn_ops(i):
        def done1(hf, j, val, rs):
            f_s[hf, j, rs] = jnp.maximum(val, 0.0)

        def done2(hf, j, val, rs):
            out_s[rows(i, hf * QB, QB), 128 * j:128 * j + 128] = val.astype(out_s.dtype)

        def init(hf, j, rs):
            return h_s[hf, rs, 128 * j:128 * j + 128]

        def add(hf, j, val, rs):
            h_s[hf, rs, 128 * j:128 * j + 128] = val

        return (units(Matmul("g1", hn_s, done1).ops(), 64) + units(Matmul("f1", hn_s, done1).ops())
                + units(Matmul("g2", f_s, add, init).ops(), 64) + units(Matmul("f2", f_s, done2, init).ops()))

    def units(ops, height=QB):
        for n, (mm, m) in enumerate(ops):
            mm.unit[m] = n // 4
        us = [("dense", [op + (slice(0, height),) for op in ops[j:j + 4]]) for j in range(0, len(ops), 4)]
        if height < QB and len(us[-1][1]) == 2:
            us[-1] = ("dense", [op + (slice(r, r + height // 2),) for r in (height // 2, 0) for op in ops[-2:]])
        return us

    def halves(us):
        return [("dense", [op[:2] + (slice(r, r + QB // 2),) for op in u]) for r in (0, QB // 2) for _, u in us]

    def with_attention(i, parts):
        seq = [("scores", i, 0)]
        for g in range(H // 2):
            seq += ([("scores", i, g + 1)] if g + 1 < H // 2 else []) + [("values", i, g)]
        plan = []
        for dense, n in parts:
            done, total = 0, sum(map(beats, dense))
            for j in range(n):
                plan.append(seq.pop(0))
                while sum(map(beats, dense[:done])) < total * (j + 1) / n - 8:
                    plan.append(dense[done])
                    done += 1
            plan += dense[done:]
        assert not seq
        return plan

    def beats(e):
        if e[0] == "dense":
            return (e[1][0][2].stop - e[1][0][2].start) // 8
        if e[0] == "call":
            return 0
        n = key_blocks(e[1], tiles(e[1], e[2])[0][0])
        return 3 * n if e[0] == "values" else (16, 32, 35)[n - 1]

    class Plan:
        def __init__(self, steps):
            self.steps = steps
            self.start = [0]
            for e in steps:
                self.start.append(self.start[-1] + beats(e))
            self.due = []

        def times(self, kind, uses=None):
            return [t for e, t in zip(self.steps, self.start)
                    if e[0] == kind and (uses is None or any(uses(mm.name, mm.prods[n][1]) for mm, n, _ in e[1]))]

        def spread(self, tasks, t0, t1):
            self.due += [(t0 + (t1 - t0) * n / len(tasks), fn) for n, fn in enumerate(tasks)]

        def sum_weights(self, name, t0, t1):
            def needed(group):
                ts = self.times("dense", lambda n, beta: n == name and beta in group[1])
                return min([t for t in ts if t > t0] + [t1 + 12]) - 12

            groups = sorted(weight_sum_tasks(name), key=needed)
            t = t1
            for group in groups[::-1]:
                t = min(t, needed(group))
                dt = (t1 - t0) * group[0] / sum(g[0] for g in groups)
                self.spread(group[2], max(t - dt, t0), max(t, t0))
                t -= dt

        def pull(self, n):
            t0, end = self.start[n], self.times("dense")[-1]
            t1 = self.start[n + 2 if [e[0] for e in self.steps[n + 1:n + 2]] == ["values"] else n + 1]
            now = sorted((w for w in self.due if min(w[0], end) < t1), key=lambda w: w[0])
            self.due = [w for w in self.due if min(w[0], end) >= t1]
            deps = [(min(max((t - t0) / (t1 - t0), 0), 0.999), dep) for t, fn in now for dep in fn()]

            def apply(lhs):
                if not deps:
                    return lhs
                vs = _split(lhs)
                for g in range(len(vs)):
                    ds = [dep for t, dep in deps if int(t * len(vs)) == g]
                    if ds:
                        vs[g] = after(functools.reduce(jnp.maximum, ds), vs[g])
                return _cat(vs)
            return apply

        def push(self, val):
            for r in range(0, val.shape[0], 8):
                if self.skip > 0:
                    self.skip -= 1
                    continue
                self.credit += self.rate
                while self.queue and self.credit >= 1:
                    self.credit -= 1
                    self.queue.pop(0)[1](val[r:r + 8])

        def scores(self, n, i, g):
            pull = self.pull(n)
            for ahead in ([g + 1] if g > 0 else [0, 1]):
                for b, h in sorted(tiles(i, ahead), key=lambda bh: bh[::-1]):
                    relayout(i, b, h, self.mark)
            dots = [score_dots(i, b, h, pull if j == 3 else (lambda v: v)) for j, (b, h) in enumerate(tiles(i, g))]
            dots = [_cat(ds) for ds in zip(*[[fn() for fn in fns] for fns in zip(*dots)])]
            tasks = []
            for j, (b, h) in enumerate(tiles(i, g)):
                if j == 3:
                    self.push(dots[j])
                tasks += softmax_tasks(i, b, dots[j], (4 * g + j) % NBUF)
            self.mark = dots[3][0:8]
            self.queue += [(g, fn) for fn in tasks]
            end, window = self.steps.index(("values", i, g)), 0
            for m in range(n + 1, end):
                if self.steps[m][0] != "values":
                    window += max(min(beats(self.steps[m]), self.start[end] - 16 - self.start[m]), 0)
                if self.steps[m][0] == "scores":
                    break
            self.skip, self.credit = 3, 0.0
            self.rate = len(self.queue) / max((window - self.skip) * 0.8, 1)

        def values(self, n, i, g):
            while self.queue and self.queue[0][0] <= g:
                self.queue.pop(0)[1](None)
            ts = tiles(i, g)
            outs = [weighted_values(i, b, h, (4 * g + j) % NBUF) for j, (b, h) in enumerate(ts)]
            for j in (0, 2):
                b, h = ts[j]
                lo, hi = normalize(h, outs[j]), normalize(h + 1, outs[j + 1])
                ot_s[b, DH * h:DH * (h + 2), :] = _cat(lo[:2] + [jnp.where(sub8 < 4, lo[2], hi[0])] + hi[1:])
                t = DH * (h + 2) // 128 - 1
                if first(i) and t >= 0 and DH * h < 128 * (t + 1):
                    self.due.append((self.start[n] + 80, partial(lambda v: v, transpose_output(i, b, t))))
            if not first(i) and g == H // 2 - 1:
                self.spread([partial(transpose_output, i, b, t, self.mark) for t in range(ND) for b in range(2)],
                            self.start[n] + 30, self.start[n] + 110)

        def run(self):
            memo.clear()
            self.queue, self.rate, self.credit, self.skip, self.mark = [], 0.0, 0.0, 0, None
            for n, e in enumerate(self.steps):
                if e[0] == "call":
                    e[1]()
                elif e[0] == "dense":
                    pull = self.pull(n)
                    for j, (mm, m, rs) in enumerate(e[1]):
                        p = mm.run(m, rs, pull if j == 0 else (lambda v: v))
                        if j == 1:
                            self.push(p)
                elif e[0] == "scores":
                    self.scores(n, e[1], e[2])
                else:
                    self.values(n, e[1], e[2])
            assert not self.due and not self.queue

    def prologue():
        for copies in (x_copies(0), x_copies(1), w_copies(0), w_copies(1), w_copies(2), w_copies(3), w_copies(4),
                       w_copies(5) + w_copies(6), w_copies(7), x_copies(2), x_copies(3)):
            for c in copies:
                c.start()
            pl.semaphore_signal(sem_order)
            pl.semaphore_wait(sem_order)
        init_query_masks()
        for i, dst in enumerate((xnext_s, xn_s)):
            wait(x_copies(i))
            for fn in ln1_tasks(i, dst):
                fn()
        wait(w_copies(0))
        v0, v1 = v_ops(0, _scheme(ND, ND)), v_ops(1, _scheme(ND, ND))
        kq0, kq1 = units(kq_ops(0, _scheme(ND, 2 * ND))), units(kq_ops(1))
        o0 = units(o_ops(0, sorted(SCHEMES["o"], key=lambda p: len(p[1]) > 1)))
        f0 = ffn_ops(0)
        a0 = with_attention(0, [(kq1[:-6], 29), (kq1[-6:-3], 2), (kq1[-3:], 1)])
        a1 = with_attention(1, [(o0, 1), ([], 2), (f0[:-8], 28), (f0[-8:], 1)])
        plan = Plan(units(v0[:10] + v1[:10]) + [("call", partial(wait, w_copies(1)))]
                    + units(v0[10:30] + v1[10:30]) + [("call", partial(wait, w_copies(2)))]
                    + units(v0[30:] + v1[30:]) + [("call", partial(wait, w_copies(3)))]
                    + kq0[:12] + [("call", partial(wait, w_copies(4)))] + kq0[12:]
                    + a0[:30] + [("call", partial(wait, w_copies(5) + w_copies(6)))] + a0[30:]
                    + a1[:22] + [("call", partial(wait, w_copies(7) + x_copies(2)))] + a1[22:])
        arrived, end = plan.times("call"), plan.start[-1]
        o_at, g1_at, f1_at, g2_at = [plan.times("dense", lambda n, _: n == name) for name in ("o", "g1", "f1", "g2")]
        plan.sum_weights("v", arrived[1], arrived[3])
        plan.sum_weights("kq", arrived[3], arrived[3] + 16 * 13)
        plan.sum_weights("f1", arrived[4] + 16, f1_at[-1])
        plan.sum_weights("g1", arrived[4] + 16, g1_at[0])
        plan.sum_weights("g2", arrived[5] + 16, g2_at[0])
        plan.sum_weights("f2", arrived[5] + 16, end - 10)
        plan.sum_weights("o", arrived[4] + 16, o_at[-1])
        plan.spread(ln2_tasks(), g1_at[0] - 30, g1_at[0])
        plan.spread(ln1_tasks(2, xn_s), end - 150, end - 10)
        plan.run()
        wait(x_copies(3))

    def step(i, carry):
        proj = units(o_ops(i - 1) + kq_ops(i) + v_ops(i))
        ffn = ffn_ops(i - 1)
        plan = Plan(proj[:2] + [("call", out_copy(i - 2).start)] + proj[2:]
                    + with_attention(i, [(ffn[:-8], 31), (ffn[-8:], 1)]))
        t0, t1 = 16 * len(proj), plan.start[-1]
        plan.spread(ln2_tasks(), 236, 600)
        plan.spread(ln1_tasks(jnp.minimum(i + 1, NSTEP - 1), xnext_s), 420, t0)
        plan.spread(advance_tasks(), t0 + 0.1 * (t1 - t0), t0 + 0.9 * (t1 - t0))
        plan.run()
        return carry

    def epilogue():
        wait([out_copy(i) for i in range(NSTEP - 2)])
        out_copy(NSTEP - 2).start()
        proj, ffn = units(o_ops(NSTEP - 1)), ffn_ops(NSTEP - 1)
        f2 = ffn[-1][1][-1][0]
        steps = halves(proj) + halves(ffn[9:17]) + ffn[:9] + ffn[17:-20]
        for n, unit in enumerate(ffn[-20:]):
            steps += [unit] + [("call", last_out_copy(j).start) for j in range(ND)
                               if min(f2.unit[f2.last[j]] + 2, 19) == n]
        plan, tasks, t = Plan(steps), ln2_tasks(), 16 * len(proj)
        plan.spread(tasks[:16], t - 16, t)
        plan.spread(tasks[16:], t + 48, t + 64)
        plan.run()
        wait([out_copy(NSTEP - 2)] + [last_out_copy(j) for j in range(ND)])

    prologue()
    lax.fori_loop(2, NSTEP, step, 0)
    epilogue()


@jax.jit
def pallas_sequential_preLN__sliding_block__dense_activation_relu__prompt_kernel(
    A_x: jax.Array,
    A_wqkv: jax.Array,
    A_wo: jax.Array,
    B_x: jax.Array,
    B_w1: jax.Array,
    B_w2: jax.Array,
):
    del B_x
    any_spec = pl.BlockSpec(memory_space=pl.ANY)
    out = pl.pallas_call(
        _kernel,
        in_specs=[any_spec] * 5,
        out_specs=any_spec,
        out_shape=jax.ShapeDtypeStruct((S, D), A_x.dtype),
        scratch_shapes=[
            pltpu.VMEM((S, D), BF16),
            pltpu.VMEM((S, D), BF16),
            pltpu.VMEM((3 * ND, D, 128), BF16),
            pltpu.VMEM((ND, D, 128), BF16),
            pltpu.VMEM((NF, D, 128), BF16),
            pltpu.VMEM((ND, DFF, 128), BF16),
            pltpu.VMEM((len(WEIGHT_SUMS), 128, 128), BF16),
            pltpu.VMEM((2, ND, QB, 128), F32),
            pltpu.VMEM((2, ND, QB, 128), F32),
            pltpu.VMEM((2, 2, ND, QB, 128), BF16),
            pltpu.VMEM((2, 2, ND, QB, 128), BF16),
            pltpu.VMEM((2, 2, ND, QB, 128), F32),
            pltpu.VMEM((RING, H, QB // 2, 128), U32),
            pltpu.VMEM((2, D // 2 + 16, 128), U32),
            pltpu.VMEM((32, 8, 128), U32),
            pltpu.VMEM((RING, D, 128), F32),
            pltpu.VMEM((NBUF, 2 * QB, 128), F32),
            pltpu.VMEM((NBUF, 2 * QB, 128), BF16),
            pltpu.VMEM((2, D, 128), F32),
            pltpu.VMEM((2, 2, ND, QB, 128), F32),
            pltpu.VMEM((2, QB, D), F32),
            pltpu.VMEM((2, ND, QB, 128), F32),
            pltpu.VMEM((2, NF, QB, 128), F32),
            pltpu.VMEM((2, NF + ND, QB, 128), F32),
            pltpu.SemaphoreType.DMA((4,)),
            pltpu.SemaphoreType.DMA((8,)),
            pltpu.SemaphoreType.DMA((NSTEP,)),
            pltpu.SemaphoreType.REGULAR,
        ],
        compiler_params=pltpu.CompilerParams(vmem_limit_bytes=100 * 1024 * 1024),
        name="fused_block",
    )(A_x.reshape(S, D), A_wqkv, A_wo, B_w1, B_w2)
    return out.reshape(A_x.shape)
```
